```python
import jax
import jax.numpy as jnp

def _softmax(x, axis=-1):
    return jax.nn.softmax(x, axis=axis)

def _gelu(x):
    return jax.nn.gelu(x, approximate=True)

def _silu(x):
    return jax.nn.silu(x)

def _sigmoid(x):
    return jax.nn.sigmoid(x)

def _layernorm(x, axis=-1, eps=1e-05):
    m = jnp.mean(x, axis=axis, keepdims=True)
    v = jnp.var(x, axis=axis, keepdims=True)
    return (x - m) / jnp.sqrt(v + eps)

def _scatter_add(tgt, idx, src, axis=0):
    return tgt.at[idx].add(src)

def _segment_sum(src, seg, n):
    return jax.ops.segment_sum(src, seg, n)

class _Rng:

    def __init__(self, key):
        self._k = key

    def _next(self):
        self._k, sub = jax.random.split(self._k)
        return sub

    def normal(self, shape):
        return jax.random.normal(self._next(), shape, dtype=jnp.bfloat16)

    def randint(self, lo, hi, shape):
        return jax.random.randint(self._next(), shape, lo, hi, dtype=jnp.int32)

    def uniform(self, shape, lo=0.0, hi=1.0):
        return jax.random.uniform(self._next(), shape, jnp.bfloat16, lo, hi)

    def permutation(self, n):
        return jax.random.permutation(self._next(), n)
kernel_name = 'interleave_layers__memory_aug_recurrent_mem_tr__glu_gated_geglu__prompt'

def setup_inputs():
    _rng = _Rng(jax.random.key(int.from_bytes(__import__("os").urandom(4), "little")))
    _w = lambda a: (lambda t: t.astype(jnp.bfloat16) if jnp.issubdtype(t.dtype, jnp.floating) else t)(jnp.asarray(a))

    def _A_setup():
        B, S, Dm = (1, 2048, 1024)
        H, Dh = (32, 128)
        M, seg = (8, 32)
        seg = min(seg, S)
        S = S // seg * seg
        return {'x': _w((lambda *s: _rng.normal(s) * 0.05)(B, S, Dm)), 'mem0': _w((lambda *s: _rng.normal(s) * 0.05)(B, M, Dm)), 'Wq': _w((lambda *s: _rng.normal(s) * 0.05)(Dm, H, Dh) * Dm ** (-0.5)), 'Wk': _w((lambda *s: _rng.normal(s) * 0.05)(Dm, H, Dh) * Dm ** (-0.5)), 'Wv': _w((lambda *s: _rng.normal(s) * 0.05)(Dm, H, Dh) * Dm ** (-0.5)), 'Wo': _w((lambda *s: _rng.normal(s) * 0.05)(H, Dh, Dm) * (H * Dh) ** (-0.5)), 'seg_len': seg}
    _A_in = _A_setup()

    def _B_setup():
        B, S, Dm, Df = (1, 2048, 1024, 3584)
        return {'x': _w((lambda *s: _rng.normal(s) * 0.05)(B, S, Dm)), 'w_gate': _w((lambda *s: _rng.normal(s) * 0.05)(Dm, Df) * Dm ** (-0.5)), 'w_up': _w((lambda *s: _rng.normal(s) * 0.05)(Dm, Df) * Dm ** (-0.5)), 'w_down': _w((lambda *s: _rng.normal(s) * 0.05)(Df, Dm) * Df ** (-0.5))}
    _B_in = _B_setup()
    return {'A_x': _A_in['x'], 'A_mem0': _A_in['mem0'], 'A_Wq': _A_in['Wq'], 'A_Wk': _A_in['Wk'], 'A_Wv': _A_in['Wv'], 'A_Wo': _A_in['Wo'], 'A_seg_len': _A_in['seg_len'], 'B_x': _B_in['x'], 'B_w_gate': _B_in['w_gate'], 'B_w_up': _B_in['w_up'], 'B_w_down': _B_in['w_down']}

def reference(A_x, A_mem0, A_Wq, A_Wk, A_Wv, A_Wo, A_seg_len, B_x, B_w_gate, B_w_up, B_w_down):

    def _A_ref(x, mem0, Wq, Wk, Wv, Wo, seg_len):
        B, S, Dm = x.shape
        H, Dh = (Wq.shape[1], Wq.shape[2])
        M = mem0.shape[1]
        scale = Dh ** (-0.5)
        n_seg = S // seg_len
        L = M + seg_len
        idx = jnp.arange(L)
        mask = (idx[:, None] < M) | (idx[:, None] >= idx[None, :])
        mem = mem0
        outs = []
        for s in range(n_seg):
            xs = x[:, s * seg_len:(s + 1) * seg_len, :].copy()
            h = jnp.concatenate([mem, xs], axis=1)
            q = jnp.einsum('btd,dhe->bhte', h, Wq)
            k = jnp.einsum('btd,dhe->bhte', h, Wk)
            v = jnp.einsum('btd,dhe->bhte', h, Wv)
            scores = jnp.einsum('bhqe,bhke->bhqk', q, k) * scale
            scores = jnp.where(mask[None, None], scores, -1000000000.0)
            p = _softmax(scores, axis=-1)
            o = jnp.einsum('bhqk,bhke->bhqe', p, v)
            o = jnp.einsum('bhte,hed->btd', o, Wo)
            mem = o[:, :M, :].copy()
            outs.append(o[:, M:, :])
        return jnp.concatenate(outs, axis=1)

    def _B_ref(x, w_gate, w_up, w_down):
        g = jnp.einsum('bsd,df->bsf', x, w_gate)
        u = jnp.einsum('bsd,df->bsf', x, w_up)
        h = _gelu(g) * u
        return jnp.einsum('bsf,fd->bsd', h, w_down)
    x = A_x
    x = x + _A_ref(_layernorm(x, axis=-1), A_mem0, A_Wq, A_Wk, A_Wv, A_Wo, A_seg_len)
    x = x + _B_ref(_layernorm(x, axis=-1), B_w_gate, B_w_up, B_w_down)
    x = x + _A_ref(_layernorm(x, axis=-1), A_mem0, A_Wq, A_Wk, A_Wv, A_Wo, A_seg_len)
    x = x + _B_ref(_layernorm(x, axis=-1), B_w_gate, B_w_up, B_w_down)
    return x
```

```python
import functools

import jax
import jax.numpy as jnp
from jax import lax
import jax.experimental.pallas as pl
import jax.experimental.pallas.tpu as pltpu

F32 = jnp.float32
BF16 = jnp.bfloat16
U32 = jnp.uint32
HG = 4
EPS = 1e-5
NEG = -1000000000.0


def _layernorm(x):
    m = jnp.mean(x, axis=-1, keepdims=True)
    c = x - m
    v = jnp.mean(c * c, axis=-1, keepdims=True)
    return c * lax.rsqrt(v + EPS)


def _dot(a, b):
    return jnp.dot(a, b, preferred_element_type=F32)


def _dot_nt(a, b):
    return lax.dot_general(a, b, (((1,), (1,)), ((), ())), preferred_element_type=F32)


def _words(x):
    return pltpu.bitcast(x.astype(BF16), U32)


def _halves(w):
    return pltpu.bitcast(w, BF16)


def _body(x_hbm, mem0_ref, wq_hbm, wk_hbm, wv_hbm, wo_hbm, wg_hbm, wu_hbm, wd_hbm, out_hbm,
          xv, ov, stage, wqkv_even, wqkv_odd, wo, wg, wu, wd, pre_in, pre, hbuf, obuf, fbuf, gbuf, dres, rbuf,
          x2buf, fill, sem_x, sem_first, sem_qkv, sem_w, sem_o, *, S, D, H, Dh, M, L, Df, cfg):
    n_seg = S // L
    NG = H // HG
    R = 2 * M + 2 * L
    RH = 2 * M + L
    GW = HG * Dh
    FC = cfg.get("FC", 512)
    NF = Df // FC
    NP = cfg.get("NP", 14)
    scale = Dh ** -0.5

    def seg(s, rows=L):
        return pl.ds(pl.multiple_of(s * rows, rows), rows)

    XA = (3 + NP) * L
    x_cp0 = pltpu.make_async_copy(x_hbm.at[0:XA], xv.at[0:XA], sem_x.at[0])
    x_cp1 = pltpu.make_async_copy(x_hbm.at[XA:S], xv.at[XA:S], sem_x.at[1])

    def qkv_copies(g):
        return [pltpu.make_async_copy(
            src.bitcast(U32).at[:, g * (HG // 2) + jj, :], stage.at[g, w * (HG // 2) + jj],
            sem_qkv.at[g])
            for w, src in enumerate((wq_hbm, wk_hbm, wv_hbm)) for jj in range(HG // 2)]

    def pieces(src, dst, n, sem0):
        rows = dst.shape[0] // n
        return [pltpu.make_async_copy(src.bitcast(U32).at[i * rows:(i + 1) * rows],
                                      dst.at[i * rows:(i + 1) * rows], sem_w.at[sem0 + i])
                for i in range(n)]

    wo_cps = pieces(wo_hbm, wo, 4, 0)
    ffn_cps = pieces(wg_hbm, wg, 2, 4) + pieces(wu_hbm, wu, 2, 6) + pieces(wd_hbm, wd, 2, 8)
    late_cps = list(zip(cfg.get("when", (0, 1, 2, 3, 4, 5, 6, 6, 7, 7, 8)), wo_cps + ffn_cps + [x_cp1]))
    x_cp0.start()
    PF = cfg.get("PF", 3)
    first_cps = [[pltpu.make_async_copy(src.bitcast(U32).at[:, jj, :], stage.at[0, w * (HG // 2) + jj],
                                        sem_first.at[w]) for jj in range(HG // 2)]
                 for w, src in enumerate((wq_hbm, wk_hbm, wv_hbm))]
    for cps in first_cps:
        for cp in cps:
            cp.start()

    row = lax.broadcasted_iota(jnp.int32, (R, R), 0)
    col = lax.broadcasted_iota(jnp.int32, (R, R), 1)
    allowed = jnp.where((row < 2 * M) | (row >= col), 0.0, NEG)
    fill[0] = jnp.where(((row >= M) & (row < RH)) == ((col >= M) & (col < RH)), allowed, -jnp.inf)
    fill[1] = jnp.where(((row >= M) & (row < 2 * M)) == ((col >= M) & (col < 2 * M)), allowed, -jnp.inf)

    def set_mem(m1, m2):
        hbuf[0:M, :] = _words(jnp.concatenate([m1, m2], axis=0))

    def x_rows(s):
        return xv[seg(s), :].astype(F32)

    x_cp0.wait()
    pre_in[...] = _words(_layernorm(xv[2 * L:(2 + NP) * L, :].astype(F32)))

    wqkv = (wqkv_even, wqkv_odd)
    n_parts = 3 * HG // 2
    RC = cfg.get('RC', 32)

    def repack(i, par, parts):
        for p in parts:
            w, jj = divmod(p, HG // 2)
            c0 = w * GW + 2 * jj * Dh
            for r in range(0, D // 2, RC):
                ev = stage[2 * i + par, p, pl.ds(2 * r, RC, stride=2), :]
                od = stage[2 * i + par, p, pl.ds(2 * r + 1, RC, stride=2), :]
                wqkv[par][i, r:r + RC, c0:c0 + Dh] = (ev & U32(0xFFFF)) | (od << 16)
                wqkv[par][i, r:r + RC, c0 + Dh:c0 + 2 * Dh] = (ev >> 16) | (od & U32(0xFFFF0000))

    def precompute(i, par, k, c0=0, c1=3 * GW):
        r = _words(_dot(_halves(pre_in[k * L:(k + 1) * L, :]), _halves(wqkv[par][i, :, c0:c1])))
        pre[2 * k, 2 * i + par, :, c0:c1] = r[:L // 2]
        pre[2 * k + 1, 2 * i + par, :, c0:c1] = r[L // 2:]

    def wait_qkv(g):
        pltpu.make_async_copy(stage.at[g], stage.at[g], sem_qkv.at[g]).wait()

    def start_late(g):
        for when, cp in late_cps:
            if isinstance(g, int):
                if when == g:
                    cp.start()
            elif 0 < when < NG - 1:
                pl.when(g == when)(cp.start)

    def load_step(i, par, first=0):
        g = 2 * i + par
        wait_qkv(g + 1)

        @pl.when(g + 2 < NG)
        def _():
            for cp in qkv_copies(g + 2):
                cp.start()
        start_late(g)
        n = NP // 2 - first
        inter = cfg.get("inter", 1)
        if inter == 2:
            repack(i + par, 1 - par, range(n_parts))
        for k in range(n):
            precompute(i, par, first + k)
            if inter == 1:
                repack(i + par, 1 - par, range(k * n_parts // n, (k + 1) * n_parts // n))
        if inter == 0:
            repack(i + par, 1 - par, range(n_parts))

    assert NP % 2 == 0
    if cfg.get("split0", 1):
        for w in range(3):
            for cp in first_cps[w]:
                cp.wait()
            if w == 1:
                for cp in qkv_copies(1):
                    cp.start()
            repack(0, 0, range(w * HG // 2, (w + 1) * HG // 2))
            for k in range(NP // 2 - PF):
                precompute(0, 0, k, w * GW, (w + 1) * GW)
        load_step(0, 0, NP // 2 - PF)
    else:
        for w in range(3):
            for cp in first_cps[w]:
                cp.wait()
        for cp in qkv_copies(1):
            cp.start()
        repack(0, 0, range(n_parts))
        for k in range(NP // 2 - PF):
            precompute(0, 0, k)
        load_step(0, 0, NP // 2 - PF)

    def load_pair(i, c):
        load_step(i, 1)
        load_step(i + 1, 0)
        return c
    lax.fori_loop(0, NG // 2 - 1, load_pair, 0)
    start_late(NG - 1)
    for k in range(NP // 2):
        precompute(NG // 2 - 1, 1, k)
    start_late(NG)

    def qkv(g, rows, pre_slot):
        n = rows if pre_slot is None else RH
        t = _dot(_halves(hbuf[0:n // 2, :]), _halves(wqkv[g % 2][g // 2])).astype(BF16)
        if pre_slot is not None:
            t = jnp.concatenate([t, _halves(pre[pre_slot, g])], axis=0)
        return t

    def scores(t):
        return [_dot_nt(t[:, i * Dh:(i + 1) * Dh], t[:, GW + i * Dh:GW + (i + 1) * Dh])
                for i in range(HG)]

    def softmax(s, which):
        n = s.shape[0]
        f = fill[which, 0:n, 0:n]
        s = jnp.where(f == 0.0, s * scale, f)
        e = jnp.exp(s - jnp.max(s, axis=-1, keepdims=True))
        l = jnp.sum(e, axis=-1, keepdims=True)
        r = pl.reciprocal(l, approx=True)
        r = r * (2.0 - l * r)
        return (e * r).astype(BF16)

    def pv(g, t, ps):
        for i, p in enumerate(ps):
            o = _dot(p, t[:, 2 * GW + i * Dh:2 * GW + (i + 1) * Dh])
            c0 = (g * HG + i) * Dh
            obuf[0:o.shape[0] // 2, c0:c0 + Dh] = _words(o)

    def ffn_in():
        fbuf[...] = _words(_layernorm(rbuf[...]))

    def gate_up(c):
        f = _halves(fbuf[...])
        a = _dot(f, _halves(wg[:, c * FC:(c + 1) * FC]))
        u = _dot(f, _halves(wu[:, c * FC:(c + 1) * FC]))
        gbuf[:, c * FC:(c + 1) * FC] = _words(jax.nn.gelu(a, approximate=True) * u)

    def down(c0, c1):
        return rbuf[:, c0:c1] + _dot(_halves(gbuf[...]), _halves(wd[:, c0:c1]))

    def attention(rows, pre_slot, which, with_ffn):
        cur = qkv(0, rows, pre_slot)
        if with_ffn:
            ffn_in()
            gate_up(0)
        late = cfg.get("late", 0)
        held = None
        for g in range(NG):
            ss = scores(cur)
            last = g + 1 == NG
            if late and held is not None:
                pv(*held)
            nxt = None if last else qkv(g + 1, rows, pre_slot)
            if with_ffn and g + 1 < NF:
                gate_up(g + 1)
            if with_ffn and last:
                dres[:, :D // 2] = down(0, D // 2)
            held = (g, cur, [softmax(s, which) for s in ss])
            if not late or last:
                pv(*held)
            cur = nxt
        if with_ffn:
            dres[:, D // 2:] = down(D // 2, D)

    def out_proj(rows):
        return _dot(_halves(obuf[0:rows // 2, :]), _halves(wo[...]))

    def single_layer_step(which, mem_slot, resid, half):
        attention(RH, None, which, False)
        a = out_proj(RH)
        rbuf[seg(half), :] = resid() + a[2 * M:RH]
        return a[mem_slot * M:(mem_slot + 1) * M]

    def ffn_step():
        ffn_in()
        for c in range(NF):
            gate_up(c)
        return down(0, D)

    def full_step(t, pre_slot, with_ffn):
        attention(R, pre_slot, 0, with_ffn)
        if with_ffn:
            d = dres[...]
            ov[seg(t - 3), :] = d[L:, :].astype(BF16)
            x2buf[(t + 1) % 2] = d[:L, :]
            x2_next = d[:L, :]
        else:
            x2_next = x2buf[(t + 1) % 2]
        hbuf[M:RH // 2, :] = _words(_layernorm(x2_next))
        hbuf[RH // 2:R // 2, :] = _words(_layernorm(x_rows(jnp.minimum(t + 1, n_seg - 1))))
        a = out_proj(R)
        set_mem(a[0:M], a[M:2 * M])
        rbuf[0:L, :] = x_rows(t) + a[RH:R]
        rbuf[L:, :] = x2buf[t % 2] + a[2 * M:RH]

    def out_copy(s, rows=L):
        return pltpu.make_async_copy(ov.at[seg(s, rows)], out_hbm.at[seg(s, rows)], sem_o)

    if cfg.get("stop") == 1:
        for _, cp in late_cps: cp.wait()
        return
    if cfg.get("stop") == 6:
        for _, cp in late_cps: cp.wait()
        return
    mem0 = mem0_ref[...].astype(F32)
    zero_mem = jnp.zeros_like(mem0)
    set_mem(mem0, zero_mem)
    for cp in wo_cps:
        cp.wait()

    def fill_step(s, c):
        hbuf[M:RH // 2, :] = _words(_layernorm(x_rows(s)))
        set_mem(single_layer_step(1, 0, lambda: x_rows(s), s), zero_mem)
        return c
    lax.fori_loop(0, 2, fill_step, 0)

    for cp in ffn_cps + [x_cp1]:
        cp.wait()
    if cfg.get("stop") == 4:
        return
    d = ffn_step()
    x2buf[0] = d[:L, :]
    x2buf[1] = d[L:, :]
    hbuf[0:M, :] = hbuf[0:M, :] | _words(jnp.concatenate([zero_mem, mem0], axis=0))
    hbuf[M:RH // 2, :] = _words(_layernorm(d[:L, :]))
    if cfg.get("stop") == 5:
        return
    full_step(2, 0, False)

    if cfg.get("stop") == 2:
        return
    def pre_loop(t, c):
        full_step(t, t - 2, True)
        out_copy(t - 3).start()
        return c
    lax.fori_loop(3, 2 + NP, pre_loop, 0)

    if cfg.get("stop") == 3:
        out_copy(0, (NP - 1) * L) if False else pltpu.make_async_copy(ov.at[0:(NP - 1) * L], out_hbm.at[0:(NP - 1) * L], sem_o).wait()
        return

    UN = cfg.get("UN", 1)
    assert (n_seg - 2 - NP) % UN == 0

    def main_loop_n(i, c):
        t0 = 2 + NP + i * UN
        for k in range(UN):
            full_step(t0 + k, None, True)
        for k in range(UN):
            out_copy(t0 + k - 3).start()
        return c
    lax.fori_loop(0, (n_seg - 2 - NP) // UN, main_loop_n, 0)

    d = ffn_step()
    ov[seg(n_seg - 3), :] = d[L:, :].astype(BF16)
    out_copy(n_seg - 3).start()
    x2buf[(n_seg - 1) % 2] = d[:L, :]
    set_mem(zero_mem, _halves(hbuf[0:M, :])[M:2 * M].astype(F32))

    def drain_step(i, c):
        s = n_seg - 2 + i
        m2 = single_layer_step(0, 1, lambda: x2buf[s % 2], i)
        set_mem(zero_mem, m2)
        hbuf[M:RH // 2, :] = _words(_layernorm(x2buf[(s + 1) % 2]))
        return c
    lax.fori_loop(0, 2, drain_step, 0)

    ov[S - 2 * L:S, :] = ffn_step().astype(BF16)
    out_copy(n_seg // 2 - 1, 2 * L).start()
    pltpu.make_async_copy(ov, out_hbm, sem_o).wait()


def build(x, mem0, Wq, Wk, Wv, Wo, L, wg, wu, wd, cfg=None):
    cfg = cfg or {}
    B, S, D = x.shape
    H, Dh = Wq.shape[1], Wq.shape[2]
    M = mem0.shape[1]
    Df = wg.shape[1]
    assert B == 1 and S % (2 * L) == 0
    R = 2 * M + 2 * L
    NG = H // HG
    NP = cfg.get("NP", 14)
    any_spec = pl.BlockSpec(memory_space=pl.ANY)
    out = pl.pallas_call(
        functools.partial(_body, S=S, D=D, H=H, Dh=Dh, M=M, L=L, Df=Df, cfg=cfg),
        out_shape=jax.ShapeDtypeStruct((S, D), x.dtype),
        in_specs=[any_spec, pl.BlockSpec(memory_space=pltpu.VMEM)] + [any_spec] * 7,
        out_specs=any_spec,
        scratch_shapes=[
            pltpu.VMEM((S, D), BF16),
            pltpu.VMEM((S, D), BF16),
            pltpu.VMEM((NG, 3 * HG // 2, D, Dh), U32),
            pltpu.VMEM((NG // 2, D // 2, 3 * HG * Dh), U32),
            pltpu.VMEM((NG // 2, D // 2, 3 * HG * Dh), U32),
            pltpu.VMEM((H * Dh // 2, D), U32),
            pltpu.VMEM((D // 2, Df), U32),
            pltpu.VMEM((D // 2, Df), U32),
            pltpu.VMEM((Df // 2, D), U32),
            pltpu.VMEM((NP * L // 2, D), U32),
            pltpu.VMEM((NP, NG, L // 2, 3 * HG * Dh), U32),
            pltpu.VMEM((R // 2, D), U32),
            pltpu.VMEM((R // 2, H * Dh), U32),
            pltpu.VMEM((L, D), U32),
            pltpu.VMEM((L, Df), U32),
            pltpu.VMEM((2 * L, D), F32),
            pltpu.VMEM((2 * L, D), F32),
            pltpu.VMEM((2, L, D), F32),
            pltpu.VMEM((2, R, R), F32),
            pltpu.SemaphoreType.DMA((2,)),
            pltpu.SemaphoreType.DMA((3,)),
            pltpu.SemaphoreType.DMA((NG,)),
            pltpu.SemaphoreType.DMA((10,)),
            pltpu.SemaphoreType.DMA,
        ],
        compiler_params=pltpu.CompilerParams(vmem_limit_bytes=124 * 2**20),
        name="rmt_geglu",
    )(x.reshape(S, D), mem0.reshape(M, D), Wq, Wk, Wv, Wo.reshape(H * Dh, D), wg, wu, wd)
    return out.reshape(B, S, D)


@functools.partial(jax.jit, static_argnames=("A_seg_len",))
def pallas_interleave_layers__memory_aug_recurrent_mem_tr__glu_gated_geglu__prompt_kernel(
    A_x: jax.Array,
    A_mem0: jax.Array,
    A_Wq: jax.Array,
    A_Wk: jax.Array,
    A_Wv: jax.Array,
    A_Wo: jax.Array,
    A_seg_len: int,
    B_x: jax.Array,
    B_w_gate: jax.Array,
    B_w_up: jax.Array,
    B_w_down: jax.Array,
):
    del B_x
    return build(A_x, A_mem0, A_Wq, A_Wk, A_Wv, A_Wo, int(A_seg_len),
                 B_w_gate, B_w_up, B_w_down, {"split0": 0, "NP": 16})
```

```python
import functools

import jax
import jax.numpy as jnp
from jax import lax
import jax.experimental.pallas as pl
import jax.experimental.pallas.tpu as pltpu

F32 = jnp.float32
BF16 = jnp.bfloat16
U32 = jnp.uint32
HG = 4
EPS = 1e-5
NEG = -1000000000.0


def _layernorm(x):
    m = jnp.mean(x, axis=-1, keepdims=True)
    c = x - m
    v = jnp.mean(c * c, axis=-1, keepdims=True)
    return c * lax.rsqrt(v + EPS)


def _dot(a, b):
    return jnp.dot(a, b, preferred_element_type=F32)


def _dot_nt(a, b):
    return lax.dot_general(a, b, (((1,), (1,)), ((), ())), preferred_element_type=F32)


def _words(x):
    return pltpu.bitcast(x.astype(BF16), U32)


def _halves(w):
    return pltpu.bitcast(w, BF16)


def _unpack(w):
    return pltpu.bitcast(w << 16, F32), pltpu.bitcast(w & U32(0xFFFF0000), F32)


def _strassen_lhs(a11, a12, a21, a22):
    return (a11 + a22, a21 + a22, a11, a22, a11 + a12, a21 - a11, a12 - a22)


def _pack(rows):
    return pltpu.bitcast(pltpu.pack_elementwise(rows, packed_dtype=BF16), U32)


def _strassen_rhs(b11, b12, b21, b22):
    def add(a, b):
        return [x + y for x, y in zip(a, b)]

    def sub(a, b):
        return [x - y for x, y in zip(a, b)]

    return (add(b11, b22), b11, sub(b12, b22), sub(b21, b11), b22, add(b11, b12), add(b21, b22))


def _strassen_out(m):
    return m[0] + m[3] - m[4] + m[6], m[2] + m[4], m[1] + m[3], m[0] - m[1] + m[2] + m[5]


def _body(x_hbm, mem0_ref, wq_hbm, wk_hbm, wv_hbm, wo_hbm, wg_hbm, wu_hbm, wd_hbm, out_hbm,
          xv, ov, stage, wqkv_even, wqkv_odd, wo, wo_sum, wgu, wgu_sum, wd, wd_sum, pre_in, pre, hbuf, obuf,
          fbuf, gbuf, facc, rbuf, x2buf, fill, sem_x, sem_qkv, sem_w, sem_o,
          *, S, D, H, Dh, M, L, Df, cfg):
    n_seg = S // L
    NG = H // HG
    R = 2 * M + 2 * L
    RH = 2 * M + L
    PW = 2 * Dh
    KO = H * Dh // 2
    FQ = Df // 4
    FC = 128
    NF = FQ // FC
    DH = D // 2
    LAG = 4
    NP = cfg["NP"]
    scale = Dh ** -0.5

    def seg(s, rows=L):
        return pl.ds(pl.multiple_of(s * rows, rows), rows)

    XA = (LAG + NP) * L
    x_cp0 = pltpu.make_async_copy(x_hbm.at[0:XA], xv.at[0:XA], sem_x.at[0])
    x_cp1 = pltpu.make_async_copy(x_hbm.at[XA:S], xv.at[XA:S], sem_x.at[1])

    def qkv_copies(g, par):
        return [pltpu.make_async_copy(src.bitcast(U32).at[:, g + side * NG, :],
                                      stage.at[par, 2 * w + side], sem_qkv.at[par])
                for w, src in enumerate((wq_hbm, wk_hbm, wv_hbm)) for side in range(2)]

    def blocks(src, dst, rows, cols, sem):
        (r0, nr), (c0, nc) = rows, cols
        return [pltpu.make_async_copy(
            src.bitcast(U32).at[r0 + i * nr:r0 + (i + 1) * nr, c0 + j * nc:c0 + (j + 1) * nc],
            dst.at[2 * i + j], sem_w.at[sem[2 * i + j]]) for i in range(2) for j in range(2)]

    wo_cps = [[cp] for cp in blocks(wo_hbm, wo, (0, KO // 2), (0, DH), range(4))]
    ffn_cps = [blocks(src, wgu.at[p, w], (0, DH // 2), (2 * p * FQ, FQ), [4 + 2 * w + p] * 4)
               for w, src in enumerate((wg_hbm, wu_hbm)) for p in range(2)]
    ffn_cps += [blocks(wd_hbm, wd.at[p], (p * FQ, FQ // 2), (0, DH), [8 + p] * 4) for p in range(2)]
    late_cps = [(when, cp) for when, cps in zip(cfg["when"], wo_cps + ffn_cps + [[x_cp1]]) for cp in cps]
    x_cp0.start()
    for cp in qkv_copies(0, 0):
        cp.start()

    row = lax.broadcasted_iota(jnp.int32, (R, R), 0)
    col = lax.broadcasted_iota(jnp.int32, (R, R), 1)
    allowed = jnp.where((row < 2 * M) | (row >= col), 0.0, NEG)
    fill[0] = jnp.where(((row >= M) & (row < RH)) == ((col >= M) & (col < RH)), allowed, -jnp.inf)
    fill[1] = jnp.where(((row >= M) & (row < 2 * M)) == ((col >= M) & (col < 2 * M)), allowed, -jnp.inf)

    def set_mem(dst, at, m1, m2):
        both = _words(m1 + m2)
        for k, part in ((1, both), (2, _words(m1)), (3, _words(m2)), (4, both)):
            dst[k, 0:M, at] = part

    def set_pair(dst, at, a1, a2, b1, b2):
        for k, part in enumerate(_strassen_lhs(a1, a2, b1, b2)):
            dst[k, M:RH // 2, at] = _words(part)

    def set_single(dst, at, a1, a2):
        for k, part in ((2, a1), (3, a2), (4, a1 + a2)):
            dst[k, M:RH // 2, at] = _words(part)

    def project(lhs, rhs, paired):
        if not paired:
            a1, a2, tot = (_halves(lhs[k]) for k in (2, 3, 4))
            return _dot(a2, rhs(3)) + _dot(tot, rhs(1)), _dot(a1, rhs(2)) + _dot(tot, rhs(4))
        m = [_dot(_halves(lhs[k] if 1 <= k <= 4 else lhs[k, M:, :]), rhs(k)) for k in range(7)]
        out = _strassen_out([v[2 * M:] if 1 <= k <= 4 else v for k, v in enumerate(m)])
        return (jnp.concatenate([m[1][:2 * M] + m[3][:2 * M], out[0], out[2]], axis=0),
                jnp.concatenate([m[2][:2 * M] + m[4][:2 * M], out[1], out[3]], axis=0))

    def x_rows(s):
        return xv[seg(s), :].astype(F32)

    x_cp0.wait()
    for k in range(NP // 2):
        y = _layernorm(xv[(LAG + 2 * k) * L:(LAG + 2 * k + 2) * L, :].astype(F32))
        for j, part in enumerate(_strassen_lhs(y[:L, :DH], y[:L, DH:], y[L:, :DH], y[L:, DH:])):
            pre_in[k, j] = _words(part)

    wqkv = (wqkv_even, wqkv_odd)
    RC = 16

    def regroup(i, par):
        for w in range(3):
            for r in range(0, DH // 2, RC):
                blocks_ = [[_unpack(stage[par, 2 * w + side,
                                          pl.ds(top * DH + 2 * r + odd, RC, stride=2), :])
                            for odd in range(2)] for top in range(2) for side in range(2)]
                for e in range(2):
                    c0 = w * PW + e * Dh
                    rows = [[blk[odd][e] for odd in range(2)] for blk in blocks_]
                    for k, part in enumerate(_strassen_rhs(*rows)):
                        wqkv[par][i, k, r:r + RC, c0:c0 + Dh] = _pack(part)

    def precompute(i, par, k):
        out = _strassen_out([_dot(_halves(pre_in[k, j]), _halves(wqkv[par][i, j])) for j in range(7)])
        for j, part in enumerate(out):
            pre[2 * k + j // 2, 2 * i + par, j % 2] = _words(part)

    def wait_qkv(par):
        pltpu.make_async_copy(stage.at[par], stage.at[par], sem_qkv.at[par]).wait()

    def start_late(g):
        for when, cp in late_cps:
            if isinstance(g, int):
                if when == g:
                    cp.start()
            elif 0 < when < NG - 1:
                pl.when(g == when)(cp.start)

    def load_step(i, par, first=0):
        g = 2 * i + par
        wait_qkv(1 - par)

        @pl.when(g + 2 < NG)
        def _():
            for cp in qkv_copies(g + 2, par):
                cp.start()
        start_late(g)
        for k in range(first, NP // 2):
            precompute(i, par, k)
        regroup(i + par, 1 - par)

    assert NP % 2 == 0
    wait_qkv(0)
    for cp in qkv_copies(1, 1):
        cp.start()
    regroup(0, 0)
    PF = min(cfg["PF"], NP // 2)
    for k in range(PF):
        precompute(0, 0, k)
    load_step(0, 0, PF)

    def load_pair(i, c):
        load_step(i, 1)
        load_step(i + 1, 0)
        return c
    lax.fori_loop(0, NG // 2 - 1, load_pair, 0)
    start_late(NG - 1)
    for k in range(NP // 2):
        precompute(NG // 2 - 1, 1, k)
    start_late(NG)

    def qkv(g, paired, pre_slot):
        t = project(hbuf, lambda k: _halves(wqkv[g % 2][g // 2, k]), paired and pre_slot is None)
        t = [v.astype(BF16) for v in t]
        if pre_slot is not None:
            t = [jnp.concatenate([v, _halves(pre[pre_slot, g, j])], axis=0) for j, v in enumerate(t)]
        return t

    def head(t, w, e):
        return t[:, w * PW + e * Dh:w * PW + (e + 1) * Dh]

    def scores(ts):
        return [_dot_nt(head(t, 0, e), head(t, 1, e)) for e in range(2) for t in ts]

    def softmax(s, which):
        n = s.shape[0]
        f = fill[which, 0:n, 0:n]
        s = jnp.where(f == 0.0, s * scale, f)
        e = jnp.exp(s - jnp.max(s, axis=-1, keepdims=True))
        l = jnp.sum(e, axis=-1, keepdims=True)
        r = pl.reciprocal(l, approx=True)
        r = r * (2.0 - l * r)
        return (e * r).astype(BF16)

    def pv(g, ts, ps, paired):
        for e in range(2):
            o1, o2 = (_dot(ps[2 * e + j], head(t, 2, e)) for j, t in enumerate(ts))
            at = slice(g * PW + e * Dh, g * PW + (e + 1) * Dh)
            set_mem(obuf, at, o1[:2 * M], o2[:2 * M])
            if paired:
                set_pair(obuf, at, o1[2 * M:RH], o2[2 * M:RH], o1[RH:], o2[RH:])
            else:
                set_single(obuf, at, o1[2 * M:], o2[2 * M:])

    def weight_sums(raw, extra, idx, r):
        parts = _strassen_rhs(*(_unpack(raw[idx + (k, r)]) for k in range(4)))
        for ref, k, j in ((extra, 0, 0), (extra, 1, 5), (extra, 2, 6), (raw, 1, 2), (raw, 2, 3)):
            ref[idx + (k, r)] = _pack(parts[j])

    def operand(raw, extra, idx, k, cols=slice(None)):
        ref, j = ((extra, 0), (raw, 0), (raw, 1), (raw, 2), (raw, 3), (extra, 1), (extra, 2))[k]
        return _halves(ref[idx + (j, slice(None), cols)])

    def prepare_ffn_weights(part):
        for r in range(0, DH // 2, 8):
            weight_sums(wgu, wgu_sum, (part // 2, part % 2), slice(r, r + 8))
        for r in range(0, FQ // 4, 16):
            weight_sums(wd, wd_sum, (part // 2,),
                        pl.ds(pl.multiple_of(part % 2 * (FQ // 4) + r, 16), 16))

    def block_product(lhs, raw, extra, idx, cols):
        return _strassen_out([_dot(_halves(lhs[k]), operand(raw, extra, idx, k, cols))
                              for k in range(7)])

    def ffn_in(q):
        y = _layernorm(rbuf[q])
        parts = _strassen_lhs(y[:2 * L, :DH], y[:2 * L, DH:], y[2 * L:, :DH], y[2 * L:, DH:])
        for i, part in enumerate(parts):
            fbuf[i] = _words(part)

    def gate_up(p, c):
        cols = slice(c * FC, (c + 1) * FC)
        gate = block_product(fbuf, wgu, wgu_sum, (p, 0), cols)
        up = block_product(fbuf, wgu, wgu_sum, (p, 1), cols)
        h = [jax.nn.gelu(a, approximate=True) * u for a, u in zip(gate, up)]
        for i, part in enumerate(_strassen_lhs(*h)):
            gbuf[i, :, cols] = _words(part)

    def down(p, q, c0, c1):
        out = block_product(gbuf, wd, wd_sum, (p,), slice(c0, c1))
        for k, part in enumerate(out):
            at = (slice(k // 2 * 2 * L, (k // 2 + 1) * 2 * L), slice(k % 2 * DH + c0, k % 2 * DH + c1))
            facc[at] = jnp.where(p == 0, rbuf[(q,) + at], facc[at]) + part

    def attention(paired, pre_slot, which, ffn=None):
        cur = qkv(0, paired, pre_slot)
        if ffn:
            ffn_in(ffn[1])
        for g in range(NG):
            ss = scores(cur)
            nxt = None if g + 1 == NG else qkv(g + 1, paired, pre_slot)
            if ffn and NG - 1 - NF <= g < NG - 1:
                gate_up(ffn[0], g - (NG - 1 - NF))
            if ffn and g == NG - 1:
                down(*ffn, 0, DH // 2)
            pv(g, cur, [softmax(s, which) for s in ss], paired)
            cur = nxt
        if ffn:
            down(*ffn, DH // 2, DH)

    def out_proj(paired):
        return jnp.concatenate(
            project(obuf, lambda k: operand(wo, wo_sum, (), k), paired), axis=1)

    every = slice(None)

    def set_tokens(t2, t1=None):
        y2 = _layernorm(t2)
        if t1 is None:
            set_single(hbuf, every, y2[:, :DH], y2[:, DH:])
        else:
            y1 = _layernorm(t1)
            set_pair(hbuf, every, y2[:, :DH], y2[:, DH:], y1[:, :DH], y1[:, DH:])

    def set_memory(m1, m2):
        m = jnp.concatenate([m1, m2], axis=0)
        set_mem(hbuf, every, m[:, :DH], m[:, DH:])

    def single_layer_step(which):
        attention(False, None, which)
        a = out_proj(False)
        return a[2 * M:RH], a[0:M], a[M:2 * M]

    def ffn_batch(q):
        def half(p, c):
            ffn_in(q)
            for k in range(NF):
                gate_up(p, k)
            down(p, q, 0, DH)
            return c
        lax.fori_loop(0, 2, half, 0)

    def x2_slot(s):
        return seg((s + 2) % 4)

    def full_step(t, pre_slot, with_ffn, next_from_pre):
        m, p = t // 2, t % 2
        q = m % 2
        attention(True, pre_slot, 0, (p, q) if with_ffn else None)
        if with_ffn:
            x2buf[seg(q, 2 * L), :] = facc[:2 * L, :]
            ov[seg((m - 3) % 4, 2 * L), :] = facc[2 * L:, :].astype(BF16)
        set_tokens(x2buf[x2_slot(t + 1 - LAG), :],
                   None if next_from_pre else x_rows(jnp.minimum(t + 1, n_seg - 1)))
        a = out_proj(True)
        set_memory(a[0:M], a[M:2 * M])
        rbuf[1 - q, seg(p), :] = x_rows(t) + a[RH:R]
        rbuf[1 - q, seg(2 + p), :] = x2buf[x2_slot(t - LAG), :] + a[2 * M:RH]

    def out_copy(s, rows=2 * L):
        return pltpu.make_async_copy(ov.at[seg(s % 4, rows)], out_hbm.at[seg(s, rows)], sem_o)

    if cfg.get("stop") == 1:
        for _, cp in late_cps: cp.wait()
        return
    if cfg.get("stop") == 6:
        for _, cp in late_cps: cp.wait()
        return
    mem0 = mem0_ref[...].astype(F32)
    zero_mem = jnp.zeros_like(mem0)
    set_memory(mem0, zero_mem)
    facc[...] = jnp.zeros(facc.shape, F32)
    for (cp,) in wo_cps:
        cp.wait()

    def prepare_wo(i, c):
        for r in range(4):
            weight_sums(wo, wo_sum, (), pl.ds(pl.multiple_of(i * 64 + r * 16, 16), 16))
        return c
    lax.fori_loop(0, KO // 2 // 64, prepare_wo, 0)

    def fill_step(s, c):
        set_tokens(x_rows(s))
        a, m1, _ = single_layer_step(1)
        rbuf[0, seg(s), :] = x_rows(s) + a
        set_memory(m1, jnp.where(s == LAG - 1, mem0_ref[...].astype(F32), 0.0))
        return c
    lax.fori_loop(0, LAG, fill_step, 0)

    for cps in ffn_cps:
        for cp in cps:
            cp.wait()
    x_cp1.wait()
    lax.fori_loop(0, 4, lambda i, c: prepare_ffn_weights(i), None)
    ffn_batch(0)
    x2buf[2 * L:, :] = facc[:2 * L, :]
    x2buf[:2 * L, :] = facc[2 * L:, :]
    set_tokens(facc[:L, :])

    def first_steps(t, c):
        full_step(t, t - LAG, False, True)
        return c
    lax.fori_loop(LAG, LAG + 2, first_steps, 0)
    if cfg.get("stop") == 2:
        return

    def steady(from_pre):
        def step(t, c):
            full_step(t, t - LAG if from_pre else None, True, from_pre)

            @pl.when(t % 2 == 1)
            def _():
                pl.when(t > LAG + 3)(lambda: out_copy(t // 2 - 4).wait())
                out_copy(t // 2 - 3).start()
            return c
        return step
    lax.fori_loop(LAG + 2, LAG + NP, steady(True), 0)
    set_tokens(x2buf[x2_slot(NP), :], x_rows(LAG + NP))
    lax.fori_loop(LAG + NP, n_seg, steady(False), 0)

    m = n_seg // 2
    q = m % 2
    ffn_batch(q)
    x2buf[q * 2 * L:(q + 1) * 2 * L, :] = facc[:2 * L, :]
    ov[seg((m - 3) % 4, 2 * L), :] = facc[2 * L:, :].astype(BF16)
    out_copy(m - 4).wait()
    out_copy(m - 3).start()
    for k in range(1, 5):
        hbuf[k, 0:M // 2, :] = jnp.zeros((M // 2, DH), U32)

    def drain_step(i, c):
        s = n_seg - LAG + i
        set_tokens(x2buf[x2_slot(s), :])
        a, _, m2 = single_layer_step(0)
        rbuf[0, seg(i), :] = x2buf[x2_slot(s), :] + a
        set_memory(zero_mem, m2)
        return c
    lax.fori_loop(0, LAG, drain_step, 0)

    ffn_batch(0)
    out_copy(m - 3).wait()
    ov[0:4 * L, :] = facc[...].astype(BF16)
    last = pltpu.make_async_copy(ov.at[0:4 * L], out_hbm.at[S - 4 * L:S], sem_o)
    last.start()
    last.wait()


def build(x, mem0, Wq, Wk, Wv, Wo, L, wg, wu, wd, cfg=None):
    cfg = {"NP": 14, "PF": 4, "when": (0, 1, 2, 3, 4, 5, 6, 6, 7, 7, 8), **(cfg or {})}
    B, S, D = x.shape
    H, Dh = Wq.shape[1], Wq.shape[2]
    M = mem0.shape[1]
    Df = wg.shape[1]
    assert B == 1 and S % (2 * L) == 0
    R = 2 * M + 2 * L
    NG = H // HG
    NP = cfg["NP"]
    FQ = Df // 4
    any_spec = pl.BlockSpec(memory_space=pl.ANY)
    out = pl.pallas_call(
        functools.partial(_body, S=S, D=D, H=H, Dh=Dh, M=M, L=L, Df=Df, cfg=cfg),
        out_shape=jax.ShapeDtypeStruct((S, D), x.dtype),
        in_specs=[any_spec, pl.BlockSpec(memory_space=pltpu.VMEM)] + [any_spec] * 7,
        out_specs=any_spec,
        scratch_shapes=[
            pltpu.VMEM((S, D), BF16),
            pltpu.VMEM((8 * L, D), BF16),
            pltpu.VMEM((2, 6, D, Dh), U32),
            pltpu.VMEM((NG // 2, 7, D // 4, 6 * Dh), U32),
            pltpu.VMEM((NG // 2, 7, D // 4, 6 * Dh), U32),
            pltpu.VMEM((4, H * Dh // 4, D // 2), U32),
            pltpu.VMEM((3, H * Dh // 4, D // 2), U32),
            pltpu.VMEM((2, 2, 4, D // 4, FQ), U32),
            pltpu.VMEM((2, 2, 3, D // 4, FQ), U32),
            pltpu.VMEM((2, 4, FQ // 2, D // 2), U32),
            pltpu.VMEM((2, 3, FQ // 2, D // 2), U32),
            pltpu.VMEM((NP // 2, 7, L // 2, D // 2), U32),
            pltpu.VMEM((NP, NG, 2, L // 2, 6 * Dh), U32),
            pltpu.VMEM((7, M + L // 2, D // 2), U32),
            pltpu.VMEM((7, M + L // 2, H * Dh // 2), U32),
            pltpu.VMEM((7, L, D // 2), U32),
            pltpu.VMEM((7, L, FQ), U32),
            pltpu.VMEM((4 * L, D), F32),
            pltpu.VMEM((2, 4 * L, D), F32),
            pltpu.VMEM((4 * L, D), F32),
            pltpu.VMEM((2, R, R), F32),
            pltpu.SemaphoreType.DMA((2,)),
            pltpu.SemaphoreType.DMA((2,)),
            pltpu.SemaphoreType.DMA((10,)),
            pltpu.SemaphoreType.DMA,
        ],
        compiler_params=pltpu.CompilerParams(vmem_limit_bytes=127 * 2**20),
        name="rmt_geglu",
    )(x.reshape(S, D), mem0.reshape(M, D), Wq, Wk, Wv, Wo.reshape(H * Dh, D), wg, wu, wd)
    return out.reshape(B, S, D)


@functools.partial(jax.jit, static_argnames=("A_seg_len",))
def pallas_interleave_layers__memory_aug_recurrent_mem_tr__glu_gated_geglu__prompt_kernel(
    A_x: jax.Array,
    A_mem0: jax.Array,
    A_Wq: jax.Array,
    A_Wk: jax.Array,
    A_Wv: jax.Array,
    A_Wo: jax.Array,
    A_seg_len: int,
    B_x: jax.Array,
    B_w_gate: jax.Array,
    B_w_up: jax.Array,
    B_w_down: jax.Array,
):
    del B_x
    return build(A_x, A_mem0, A_Wq, A_Wk, A_Wv, A_Wo, int(A_seg_len),
                 B_w_gate, B_w_up, B_w_down, {"NP": 12})
```

```python
import functools

import jax
import jax.numpy as jnp
from jax import lax
import jax.experimental.pallas as pl
import jax.experimental.pallas.tpu as pltpu

F32 = jnp.float32
BF16 = jnp.bfloat16
U32 = jnp.uint32
HG = 4
EPS = 1e-5
NEG = -1000000000.0


def _layernorm(x):
    m = jnp.mean(x, axis=-1, keepdims=True)
    c = x - m
    v = jnp.mean(c * c, axis=-1, keepdims=True)
    return c * lax.rsqrt(v + EPS)


def _dot(a, b):
    return jnp.dot(a, b, preferred_element_type=F32)


def _dot_nt(a, b):
    return lax.dot_general(a, b, (((1,), (1,)), ((), ())), preferred_element_type=F32)


def _words(x):
    return pltpu.bitcast(x.astype(BF16), U32)


def _halves(w):
    return pltpu.bitcast(w, BF16)


def _unpack(w):
    return pltpu.bitcast(w << 16, F32), pltpu.bitcast(w & U32(0xFFFF0000), F32)


def _strassen_lhs(a11, a12, a21, a22):
    return (a11 + a22, a21 + a22, a11, a22, a11 + a12, a21 - a11, a12 - a22)


def _pack(rows):
    return pltpu.bitcast(pltpu.pack_elementwise(rows, packed_dtype=BF16), U32)


def _strassen_rhs(b11, b12, b21, b22):
    def add(a, b):
        return [x + y for x, y in zip(a, b)]

    def sub(a, b):
        return [x - y for x, y in zip(a, b)]

    return (add(b11, b22), b11, sub(b12, b22), sub(b21, b11), b22, add(b11, b12), add(b21, b22))


def _strassen_out(m):
    return m[0] + m[3] - m[4] + m[6], m[2] + m[4], m[1] + m[3], m[0] - m[1] + m[2] + m[5]


def _body(x_hbm, mem0_ref, wq_hbm, wk_hbm, wv_hbm, wo_hbm, wg_hbm, wu_hbm, wd_hbm, out_hbm,
          xv, ov, stage, wqkv_even, wqkv_odd, wo, wo_sum, wgu, wgu_sum, wd, wd_sum, pre_in, pre, hbuf, obuf,
          fbuf, gbuf, facc, rbuf, x2buf, fill, sem_x, sem_qkv, sem_w, sem_o,
          *, S, D, H, Dh, M, L, Df, cfg):
    n_seg = S // L
    NG = H // HG
    R = 2 * M + 2 * L
    RH = 2 * M + L
    PW = 2 * Dh
    KO = H * Dh // 2
    FQ = Df // 4
    FC = 128
    NF = FQ // FC
    DH = D // 2
    LAG = 2
    NP = cfg["NP"]
    scale = Dh ** -0.5

    def seg(s, rows=L):
        return pl.ds(pl.multiple_of(s * rows, rows), rows)

    XA = (LAG + NP) * L
    x_cp0 = pltpu.make_async_copy(x_hbm.at[0:XA], xv.at[0:XA], sem_x.at[0])
    x_cp1 = pltpu.make_async_copy(x_hbm.at[XA:S], xv.at[XA:S], sem_x.at[1])

    def qkv_copies(g, par):
        return [pltpu.make_async_copy(src.bitcast(U32).at[:, g + side * NG, :],
                                      stage.at[par, 2 * w + side], sem_qkv.at[par])
                for w, src in enumerate((wq_hbm, wk_hbm, wv_hbm)) for side in range(2)]

    def blocks(src, dst, rows, cols, sem):
        (r0, nr), (c0, nc) = rows, cols
        return [pltpu.make_async_copy(
            src.bitcast(U32).at[r0 + i * nr:r0 + (i + 1) * nr, c0 + j * nc:c0 + (j + 1) * nc],
            dst.at[2 * i + j], sem_w.at[sem[2 * i + j]]) for i in range(2) for j in range(2)]

    wo_cps = [[cp] for cp in blocks(wo_hbm, wo, (0, KO // 2), (0, DH), range(4))]
    ffn_cps = [blocks(src, wgu.at[p, w], (0, DH // 2), (2 * p * FQ, FQ), [4 + 2 * w + p] * 4)
               for w, src in enumerate((wg_hbm, wu_hbm)) for p in range(2)]
    ffn_cps += [blocks(wd_hbm, wd.at[p], (p * FQ, FQ // 2), (0, DH), [8 + p] * 4) for p in range(2)]
    late_cps = [(when, cp) for when, cps in zip(cfg["when"], wo_cps + ffn_cps + [[x_cp1]]) for cp in cps]
    x_cp0.start()
    for cp in qkv_copies(0, 0):
        cp.start()

    row = lax.broadcasted_iota(jnp.int32, (R, R), 0)
    col = lax.broadcasted_iota(jnp.int32, (R, R), 1)
    allowed = jnp.where((row < 2 * M) | (row >= col), 0.0, NEG)
    fill[0] = jnp.where(((row >= M) & (row < RH)) == ((col >= M) & (col < RH)), allowed, -jnp.inf)
    fill[1] = jnp.where(((row >= M) & (row < 2 * M)) == ((col >= M) & (col < 2 * M)), allowed, -jnp.inf)

    def set_mem(dst, at, m1, m2):
        both = _words(m1 + m2)
        for k, part in ((1, both), (2, _words(m1)), (3, _words(m2)), (4, both)):
            dst[k, 0:M, at] = part

    def set_pair(dst, at, a1, a2, b1, b2):
        for k, part in enumerate(_strassen_lhs(a1, a2, b1, b2)):
            dst[k, M:RH // 2, at] = _words(part)

    def set_single(dst, at, a1, a2):
        for k, part in ((2, a1), (3, a2), (4, a1 + a2)):
            dst[k, M:RH // 2, at] = _words(part)

    def project(lhs, rhs, paired):
        if not paired:
            a1, a2, tot = (_halves(lhs[k]) for k in (2, 3, 4))
            return _dot(a2, rhs(3)) + _dot(tot, rhs(1)), _dot(a1, rhs(2)) + _dot(tot, rhs(4))
        m = [_dot(_halves(lhs[k] if 1 <= k <= 4 else lhs[k, M:, :]), rhs(k)) for k in range(7)]
        out = _strassen_out([v[2 * M:] if 1 <= k <= 4 else v for k, v in enumerate(m)])
        return (jnp.concatenate([m[1][:2 * M] + m[3][:2 * M], out[0], out[2]], axis=0),
                jnp.concatenate([m[2][:2 * M] + m[4][:2 * M], out[1], out[3]], axis=0))

    def x_rows(s):
        return xv[seg(s), :].astype(F32)

    x_cp0.wait()
    for k in range(NP // 2):
        y = _layernorm(xv[(LAG + 2 * k) * L:(LAG + 2 * k + 2) * L, :].astype(F32))
        for j, part in enumerate(_strassen_lhs(y[:L, :DH], y[:L, DH:], y[L:, :DH], y[L:, DH:])):
            pre_in[k, j] = _words(part)

    wqkv = (wqkv_even, wqkv_odd)
    RC = 16

    def regroup(i, par):
        for w in range(3):
            for r in range(0, DH // 2, RC):
                blocks_ = [[_unpack(stage[par, 2 * w + side,
                                          pl.ds(top * DH + 2 * r + odd, RC, stride=2), :])
                            for odd in range(2)] for top in range(2) for side in range(2)]
                for e in range(2):
                    c0 = w * PW + e * Dh
                    rows = [[blk[odd][e] for odd in range(2)] for blk in blocks_]
                    for k, part in enumerate(_strassen_rhs(*rows)):
                        wqkv[par][i, k, r:r + RC, c0:c0 + Dh] = _pack(part)

    def precompute(i, par, k):
        out = _strassen_out([_dot(_halves(pre_in[k, j]), _halves(wqkv[par][i, j])) for j in range(7)])
        for j, part in enumerate(out):
            pre[2 * k + j // 2, 2 * i + par, j % 2] = _words(part)

    def wait_qkv(par):
        pltpu.make_async_copy(stage.at[par], stage.at[par], sem_qkv.at[par]).wait()

    def start_late(g):
        for when, cp in late_cps:
            if isinstance(g, int):
                if when == g:
                    cp.start()
            elif 0 < when < NG - 1:
                pl.when(g == when)(cp.start)

    def load_step(i, par, first=0):
        g = 2 * i + par
        wait_qkv(1 - par)

        @pl.when(g + 2 < NG)
        def _():
            for cp in qkv_copies(g + 2, par):
                cp.start()
        start_late(g)
        for k in range(first, NP // 2):
            precompute(i, par, k)
        regroup(i + par, 1 - par)

    assert NP % 2 == 0
    wait_qkv(0)
    for cp in qkv_copies(1, 1):
        cp.start()
    regroup(0, 0)
    PF = min(cfg["PF"], NP // 2)
    for k in range(PF):
        precompute(0, 0, k)
    load_step(0, 0, PF)

    def load_pair(i, c):
        load_step(i, 1)
        load_step(i + 1, 0)
        return c
    lax.fori_loop(0, NG // 2 - 1, load_pair, 0)
    start_late(NG - 1)
    for k in range(NP // 2):
        precompute(NG // 2 - 1, 1, k)
    start_late(NG)

    def qkv(g, paired, pre_slot):
        t = project(hbuf, lambda k: _halves(wqkv[g % 2][g // 2, k]), paired and pre_slot is None)
        t = [v.astype(BF16) for v in t]
        if pre_slot is not None:
            t = [jnp.concatenate([v, _halves(pre[pre_slot, g, j])], axis=0) for j, v in enumerate(t)]
        return t

    def head(t, w, e):
        return t[:, w * PW + e * Dh:w * PW + (e + 1) * Dh]

    def scores(ts):
        return [_dot_nt(head(t, 0, e), head(t, 1, e)) for e in range(2) for t in ts]

    def softmax(s, which):
        n = s.shape[0]
        f = fill[which, 0:n, 0:n]
        s = jnp.where(f == 0.0, s * scale, f)
        e = jnp.exp(s - jnp.max(s, axis=-1, keepdims=True))
        l = jnp.sum(e, axis=-1, keepdims=True)
        r = pl.reciprocal(l, approx=True)
        r = r * (2.0 - l * r)
        return (e * r).astype(BF16)

    def pv(g, ts, ps, paired):
        for e in range(2):
            o1, o2 = (_dot(ps[2 * e + j], head(t, 2, e)) for j, t in enumerate(ts))
            at = slice(g * PW + e * Dh, g * PW + (e + 1) * Dh)
            set_mem(obuf, at, o1[:2 * M], o2[:2 * M])
            if paired:
                set_pair(obuf, at, o1[2 * M:RH], o2[2 * M:RH], o1[RH:], o2[RH:])
            else:
                set_single(obuf, at, o1[2 * M:], o2[2 * M:])

    def weight_sums(raw, extra, idx, r):
        parts = _strassen_rhs(*(_unpack(raw[idx + (k, r)]) for k in range(4)))
        for ref, k, j in ((extra, 0, 0), (extra, 1, 5), (extra, 2, 6), (raw, 1, 2), (raw, 2, 3)):
            ref[idx + (k, r)] = _pack(parts[j])

    def operand(raw, extra, idx, k, cols=slice(None)):
        ref, j = ((extra, 0), (raw, 0), (raw, 1), (raw, 2), (raw, 3), (extra, 1), (extra, 2))[k]
        return _halves(ref[idx + (j, slice(None), cols)])

    def prepare_ffn_weights(part):
        for r in range(0, DH // 2, 8):
            weight_sums(wgu, wgu_sum, (part // 2, part % 2), slice(r, r + 8))
        for r in range(0, FQ // 4, 16):
            weight_sums(wd, wd_sum, (part // 2,),
                        pl.ds(pl.multiple_of(part % 2 * (FQ // 4) + r, 16), 16))

    def block_product(lhs, raw, extra, idx, cols):
        return _strassen_out([_dot(_halves(lhs[k]), operand(raw, extra, idx, k, cols))
                              for k in range(7)])

    def ffn_in():
        y = _layernorm(rbuf[...])
        parts = _strassen_lhs(y[:L, :DH], y[:L, DH:], y[L:, :DH], y[L:, DH:])
        for i, part in enumerate(parts):
            fbuf[i] = _words(part)

    def gate_up(chunk):
        p, c = divmod(chunk, NF)
        cols = slice(c * FC, (c + 1) * FC)
        gate = block_product(fbuf, wgu, wgu_sum, (p, 0), cols)
        up = block_product(fbuf, wgu, wgu_sum, (p, 1), cols)
        h = [jax.nn.gelu(a, approximate=True) * u for a, u in zip(gate, up)]
        for i, part in enumerate(_strassen_lhs(*h)):
            gbuf[i, :, p * FQ + c * FC:p * FQ + (c + 1) * FC] = _words(part)

    def down(c0, c1):
        out = _strassen_out([
            _dot(_halves(gbuf[k, :, 0:FQ]), operand(wd, wd_sum, (0,), k, slice(c0, c1)))
            + _dot(_halves(gbuf[k, :, FQ:]), operand(wd, wd_sum, (1,), k, slice(c0, c1)))
            for k in range(7)])
        for k, part in enumerate(out):
            at = (slice(k // 2 * L, (k // 2 + 1) * L), slice(k % 2 * DH + c0, k % 2 * DH + c1))
            facc[at] = rbuf[at] + part

    def attention(paired, pre_slot, which, with_ffn=False):
        cur = qkv(0, paired, pre_slot)
        if with_ffn:
            ffn_in()
        for g in range(NG):
            ss = scores(cur)
            nxt = None if g + 1 == NG else qkv(g + 1, paired, pre_slot)
            if with_ffn and g + 1 < NG:
                for chunk in range(g * 2 * NF // (NG - 1), (g + 1) * 2 * NF // (NG - 1)):
                    gate_up(chunk)
            elif with_ffn:
                down(0, DH // 2)
            pv(g, cur, [softmax(s, which) for s in ss], paired)
            cur = nxt
        if with_ffn:
            down(DH // 2, DH)

    def out_proj(paired):
        return jnp.concatenate(
            project(obuf, lambda k: operand(wo, wo_sum, (), k), paired), axis=1)

    every = slice(None)

    def set_tokens(t2, t1=None):
        y2 = _layernorm(t2)
        if t1 is None:
            set_single(hbuf, every, y2[:, :DH], y2[:, DH:])
        else:
            y1 = _layernorm(t1)
            set_pair(hbuf, every, y2[:, :DH], y2[:, DH:], y1[:, :DH], y1[:, DH:])

    def set_memory(m1, m2):
        m = jnp.concatenate([m1, m2], axis=0)
        set_mem(hbuf, every, m[:, :DH], m[:, DH:])

    def single_layer_step(which):
        attention(False, None, which)
        a = out_proj(False)
        return a[2 * M:RH], a[0:M], a[M:2 * M]

    def ffn_step():
        ffn_in()
        for chunk in range(2 * NF):
            gate_up(chunk)
        down(0, DH)

    def full_step(t, pre_slot, with_ffn, next_from_pre):
        attention(True, pre_slot, 0, with_ffn)
        if with_ffn:
            x2buf[(t + 1) % 2] = facc[:L, :]
            ov[(t - 3) % 2] = facc[L:, :].astype(BF16)
        set_tokens(x2buf[(t + 1) % 2],
                   None if next_from_pre else x_rows(jnp.minimum(t + 1, n_seg - 1)))
        a = out_proj(True)
        set_memory(a[0:M], a[M:2 * M])
        rbuf[0:L, :] = x_rows(t) + a[RH:R]
        rbuf[L:, :] = x2buf[t % 2] + a[2 * M:RH]

    def out_copy(s):
        return pltpu.make_async_copy(ov.at[s % 2], out_hbm.at[seg(s)], sem_o)

    mem0 = mem0_ref[...].astype(F32)
    zero_mem = jnp.zeros_like(mem0)
    set_memory(mem0, zero_mem)
    for (cp,) in wo_cps:
        cp.wait()

    def prepare_wo(i, c):
        for r in range(4):
            weight_sums(wo, wo_sum, (), pl.ds(pl.multiple_of(i * 64 + r * 16, 16), 16))
        return c
    lax.fori_loop(0, KO // 2 // 64, prepare_wo, 0)

    def fill_step(s, c):
        set_tokens(x_rows(s))
        a, m1, _ = single_layer_step(1)
        rbuf[seg(s), :] = x_rows(s) + a
        set_memory(m1, jnp.where(s == LAG - 1, mem0_ref[...].astype(F32), 0.0))
        return c
    lax.fori_loop(0, LAG, fill_step, 0)

    for cps in ffn_cps:
        for cp in cps:
            cp.wait()
    x_cp1.wait()
    lax.fori_loop(0, 4, lambda i, c: prepare_ffn_weights(i), None)
    ffn_step()
    x2buf[0] = facc[:L, :]
    x2buf[1] = facc[L:, :]
    set_tokens(facc[:L, :])
    full_step(LAG, 0, False, True)

    def steady(from_pre):
        def step(t, c):
            full_step(t, t - LAG if from_pre else None, True, from_pre)
            pl.when(t > LAG + 1)(lambda: out_copy(t - 4).wait())
            out_copy(t - 3).start()
            return c
        return step
    lax.fori_loop(LAG + 1, LAG + NP, steady(True), 0)
    set_tokens(x2buf[NP % 2], x_rows(LAG + NP))
    lax.fori_loop(LAG + NP, n_seg, steady(False), 0)

    ffn_step()
    x2buf[(n_seg - 1) % 2] = facc[:L, :]
    ov[(n_seg - 3) % 2] = facc[L:, :].astype(BF16)
    out_copy(n_seg - 4).wait()
    out_copy(n_seg - 3).start()
    for k in range(1, 5):
        hbuf[k, 0:M // 2, :] = jnp.zeros((M // 2, DH), U32)

    def drain_step(i, c):
        s = n_seg - LAG + i
        set_tokens(x2buf[s % 2])
        a, _, m2 = single_layer_step(0)
        rbuf[seg(i), :] = x2buf[s % 2] + a
        set_memory(zero_mem, m2)
        return c
    lax.fori_loop(0, LAG, drain_step, 0)

    ffn_step()
    out_copy(n_seg - 3).wait()
    ov[0] = facc[:L, :].astype(BF16)
    ov[1] = facc[L:, :].astype(BF16)
    out_copy(n_seg - 2).start()
    out_copy(n_seg - 1).start()
    out_copy(n_seg - 2).wait()
    out_copy(n_seg - 1).wait()


def build(x, mem0, Wq, Wk, Wv, Wo, L, wg, wu, wd, cfg=None):
    cfg = {"NP": 12, "PF": 4, "when": (0, 1, 2, 3, 4, 5, 6, 6, 7, 7, 8), **(cfg or {})}
    B, S, D = x.shape
    H, Dh = Wq.shape[1], Wq.shape[2]
    M = mem0.shape[1]
    Df = wg.shape[1]
    assert B == 1 and S % (2 * L) == 0
    R = 2 * M + 2 * L
    NG = H // HG
    NP = cfg["NP"]
    FQ = Df // 4
    any_spec = pl.BlockSpec(memory_space=pl.ANY)
    out = pl.pallas_call(
        functools.partial(_body, S=S, D=D, H=H, Dh=Dh, M=M, L=L, Df=Df, cfg=cfg),
        out_shape=jax.ShapeDtypeStruct((S, D), x.dtype),
        in_specs=[any_spec, pl.BlockSpec(memory_space=pltpu.VMEM)] + [any_spec] * 7,
        out_specs=any_spec,
        scratch_shapes=[
            pltpu.VMEM((S, D), BF16),
            pltpu.VMEM((2, L, D), BF16),
            pltpu.VMEM((2, 6, D, Dh), U32),
            pltpu.VMEM((NG // 2, 7, D // 4, 6 * Dh), U32),
            pltpu.VMEM((NG // 2, 7, D // 4, 6 * Dh), U32),
            pltpu.VMEM((4, H * Dh // 4, D // 2), U32),
            pltpu.VMEM((3, H * Dh // 4, D // 2), U32),
            pltpu.VMEM((2, 2, 4, D // 4, FQ), U32),
            pltpu.VMEM((2, 2, 3, D // 4, FQ), U32),
            pltpu.VMEM((2, 4, FQ // 2, D // 2), U32),
            pltpu.VMEM((2, 3, FQ // 2, D // 2), U32),
            pltpu.VMEM((NP // 2, 7, L // 2, D // 2), U32),
            pltpu.VMEM((NP, NG, 2, L // 2, 6 * Dh), U32),
            pltpu.VMEM((7, M + L // 2, D // 2), U32),
            pltpu.VMEM((7, M + L // 2, H * Dh // 2), U32),
            pltpu.VMEM((7, L // 2, D // 2), U32),
            pltpu.VMEM((7, L // 2, Df // 2), U32),
            pltpu.VMEM((2 * L, D), F32),
            pltpu.VMEM((2 * L, D), F32),
            pltpu.VMEM((2, L, D), F32),
            pltpu.VMEM((2, R, R), F32),
            pltpu.SemaphoreType.DMA((2,)),
            pltpu.SemaphoreType.DMA((2,)),
            pltpu.SemaphoreType.DMA((10,)),
            pltpu.SemaphoreType.DMA,
        ],
        compiler_params=pltpu.CompilerParams(vmem_limit_bytes=127 * 2**20),
        name="rmt_geglu",
    )(x.reshape(S, D), mem0.reshape(M, D), Wq, Wk, Wv, Wo.reshape(H * Dh, D), wg, wu, wd)
    return out.reshape(B, S, D)


@functools.partial(jax.jit, static_argnames=("A_seg_len",))
def pallas_interleave_layers__memory_aug_recurrent_mem_tr__glu_gated_geglu__prompt_kernel(
    A_x: jax.Array,
    A_mem0: jax.Array,
    A_Wq: jax.Array,
    A_Wk: jax.Array,
    A_Wv: jax.Array,
    A_Wo: jax.Array,
    A_seg_len: int,
    B_x: jax.Array,
    B_w_gate: jax.Array,
    B_w_up: jax.Array,
    B_w_down: jax.Array,
):
    del B_x
    return build(A_x, A_mem0, A_Wq, A_Wk, A_Wv, A_Wo, int(A_seg_len),
                 B_w_gate, B_w_up, B_w_down, {"NP": 14})
```

```python
import functools

import jax
import jax.numpy as jnp
from jax import lax
import jax.experimental.pallas as pl
import jax.experimental.pallas.tpu as pltpu

F32 = jnp.float32
BF16 = jnp.bfloat16
U32 = jnp.uint32
HG = 4
EPS = 1e-5
NEG = -1000000000.0


def _layernorm(x):
    m = jnp.mean(x, axis=-1, keepdims=True)
    c = x - m
    v = jnp.mean(c * c, axis=-1, keepdims=True)
    return c * lax.rsqrt(v + EPS)


def _dot(a, b):
    return jnp.dot(a, b, preferred_element_type=F32)


def _dot_nt(a, b):
    return lax.dot_general(a, b, (((1,), (1,)), ((), ())), preferred_element_type=F32)


def _words(x):
    return pltpu.bitcast(x.astype(BF16), U32)


def _halves(w):
    return pltpu.bitcast(w, BF16)


def _unpack(w):
    return pltpu.bitcast(w << 16, F32), pltpu.bitcast(w & U32(0xFFFF0000), F32)


def _strassen_lhs(a11, a12, a21, a22):
    return (a11 + a22, a21 + a22, a11, a22, a11 + a12, a21 - a11, a12 - a22)


def _pack(rows):
    return pltpu.bitcast(pltpu.pack_elementwise(rows, packed_dtype=BF16), U32)


def _strassen_rhs(b11, b12, b21, b22):
    def add(a, b):
        return [x + y for x, y in zip(a, b)]

    def sub(a, b):
        return [x - y for x, y in zip(a, b)]

    return (add(b11, b22), b11, sub(b12, b22), sub(b21, b11), b22, add(b11, b12), add(b21, b22))


def _strassen_out(m):
    return m[0] + m[3] - m[4] + m[6], m[2] + m[4], m[1] + m[3], m[0] - m[1] + m[2] + m[5]


def _body(x_hbm, mem0_ref, wq_hbm, wk_hbm, wv_hbm, wo_hbm, wg_hbm, wu_hbm, wd_hbm, out_hbm,
          xv, ov, stage, wqkv_even, wqkv_odd, wo, wo_sum, wgu, wgu_sum, wd, wd_sum, pre_in, pre, hbuf, obuf,
          fbuf, gbuf, facc, rbuf, x2buf, fill, sem_x, sem_qkv, sem_w, sem_o,
          *, S, D, H, Dh, M, L, Df, cfg):
    n_seg = S // L
    NG = H // HG
    R = 2 * M + 2 * L
    RH = 2 * M + L
    PW = 2 * Dh
    KO = H * Dh // 2
    FQ = Df // 4
    FC = 128
    NF = FQ // FC
    DH = D // 2
    LAG = 2
    NP = cfg["NP"]
    scale = Dh ** -0.5

    def seg(s, rows=L):
        return pl.ds(pl.multiple_of(s * rows, rows), rows)

    XA = (LAG + NP) * L
    x_cp0 = pltpu.make_async_copy(x_hbm.at[0:XA], xv.at[0:XA], sem_x.at[0])
    x_cp1 = pltpu.make_async_copy(x_hbm.at[XA:S], xv.at[XA:S], sem_x.at[1])

    def qkv_copies(g, par):
        return [pltpu.make_async_copy(src.bitcast(U32).at[:, g + side * NG, :],
                                      stage.at[par, 2 * w + side], sem_qkv.at[par])
                for w, src in enumerate((wq_hbm, wk_hbm, wv_hbm)) for side in range(2)]

    def blocks(src, dst, rows, cols, sem):
        (r0, nr), (c0, nc) = rows, cols
        return [pltpu.make_async_copy(
            src.bitcast(U32).at[r0 + i * nr:r0 + (i + 1) * nr, c0 + j * nc:c0 + (j + 1) * nc],
            dst.at[2 * i + j], sem_w.at[sem[2 * i + j]]) for i in range(2) for j in range(2)]

    wo_cps = [[cp] for cp in blocks(wo_hbm, wo, (0, KO // 2), (0, DH), range(4))]
    ffn_cps = [blocks(src, wgu.at[p, w], (0, DH // 2), (2 * p * FQ, FQ), [4 + 2 * w + p] * 4)
               for w, src in enumerate((wg_hbm, wu_hbm)) for p in range(2)]
    ffn_cps += [blocks(wd_hbm, wd.at[p], (p * FQ, FQ // 2), (0, DH), [8 + p] * 4) for p in range(2)]
    late_cps = [(when, cp) for when, cps in zip(cfg["when"], wo_cps + ffn_cps + [[x_cp1]]) for cp in cps]
    x_cp0.start()
    for cp in qkv_copies(0, 0):
        cp.start()

    row = lax.broadcasted_iota(jnp.int32, (R, R), 0)
    col = lax.broadcasted_iota(jnp.int32, (R, R), 1)
    allowed = jnp.where((row < 2 * M) | (row >= col), 0.0, NEG)
    fill[0] = jnp.where(((row >= M) & (row < RH)) == ((col >= M) & (col < RH)), allowed, -jnp.inf)
    fill[1] = jnp.where(((row >= M) & (row < 2 * M)) == ((col >= M) & (col < 2 * M)), allowed, -jnp.inf)

    def set_mem(dst, at, m1, m2):
        both = _words(m1 + m2)
        for k, part in ((1, both), (2, _words(m1)), (3, _words(m2)), (4, both)):
            dst[k, 0:M, at] = part

    def set_pair(dst, at, a1, a2, b1, b2):
        for k, part in enumerate(_strassen_lhs(a1, a2, b1, b2)):
            dst[k, M:RH // 2, at] = _words(part)

    def set_single(dst, at, a1, a2):
        for k, part in ((2, a1), (3, a2), (4, a1 + a2)):
            dst[k, M:RH // 2, at] = _words(part)

    def project(lhs, rhs, paired):
        if not paired:
            a1, a2, tot = (_halves(lhs[k]) for k in (2, 3, 4))
            return _dot(a2, rhs(3)) + _dot(tot, rhs(1)), _dot(a1, rhs(2)) + _dot(tot, rhs(4))
        m = [_dot(_halves(lhs[k] if 1 <= k <= 4 else lhs[k, M:, :]), rhs(k)) for k in range(7)]
        out = _strassen_out([v[2 * M:] if 1 <= k <= 4 else v for k, v in enumerate(m)])
        return (jnp.concatenate([m[1][:2 * M] + m[3][:2 * M], out[0], out[2]], axis=0),
                jnp.concatenate([m[2][:2 * M] + m[4][:2 * M], out[1], out[3]], axis=0))

    def x_rows(s):
        return xv[seg(s), :].astype(F32)

    x_cp0.wait()
    for k in range(NP // 2):
        y = _layernorm(xv[(LAG + 2 * k) * L:(LAG + 2 * k + 2) * L, :].astype(F32))
        for j, part in enumerate(_strassen_lhs(y[:L, :DH], y[:L, DH:], y[L:, :DH], y[L:, DH:])):
            pre_in[k, j] = _words(part)

    wqkv = (wqkv_even, wqkv_odd)
    RC = 16

    def regroup(i, par, which=range(3)):
        for w in which:
            for r in range(0, DH // 2, RC):
                blocks_ = [[_unpack(stage[par, 2 * w + side,
                                          pl.ds(top * DH + 2 * r + odd, RC, stride=2), :])
                            for odd in range(2)] for top in range(2) for side in range(2)]
                for e in range(2):
                    c0 = w * PW + e * Dh
                    rows = [[blk[odd][e] for odd in range(2)] for blk in blocks_]
                    for k, part in enumerate(_strassen_rhs(*rows)):
                        wqkv[par][i, k, r:r + RC, c0:c0 + Dh] = _pack(part)

    def precompute(i, par, k):
        out = _strassen_out([_dot(_halves(pre_in[k, j]), _halves(wqkv[par][i, j])) for j in range(7)])
        for j, part in enumerate(out):
            pre[2 * k + j // 2, 2 * i + par, j % 2] = _words(part)

    def wait_qkv(par):
        pltpu.make_async_copy(stage.at[par], stage.at[par], sem_qkv.at[par]).wait()

    def start_late(g):
        for when, cp in late_cps:
            if isinstance(g, int):
                if when == g:
                    cp.start()
            elif 0 < when < NG - 1:
                pl.when(g == when)(cp.start)

    def load_step(i, par, first=0):
        g = 2 * i + par
        wait_qkv(1 - par)

        @pl.when(g + 2 < NG)
        def _():
            for cp in qkv_copies(g + 2, par):
                cp.start()
        start_late(g)
        for k in range(first, NP // 2):
            precompute(i, par, k)
            if True and (k - first) % 2 == 1 and (k - first) // 2 < 3:
                regroup(i + par, 1 - par, [(k - first) // 2])
        done = (NP // 2 - first) // 2
        regroup(i + par, 1 - par, range(done, 3))

    assert NP % 2 == 0
    wait_qkv(0)
    for cp in qkv_copies(1, 1):
        cp.start()
    regroup(0, 0)
    PF = min(cfg["PF"], NP // 2)
    for k in range(PF):
        precompute(0, 0, k)
    load_step(0, 0, PF)

    def load_pair(i, c):
        load_step(i, 1)
        load_step(i + 1, 0)
        return c
    lax.fori_loop(0, NG // 2 - 1, load_pair, 0)
    start_late(NG - 1)
    for k in range(NP // 2):
        precompute(NG // 2 - 1, 1, k)
    start_late(NG)

    def qkv(g, paired, pre_slot):
        t = project(hbuf, lambda k: _halves(wqkv[g % 2][g // 2, k]), paired and pre_slot is None)
        t = [v.astype(BF16) for v in t]
        if pre_slot is not None:
            t = [jnp.concatenate([v, _halves(pre[pre_slot, g, j])], axis=0) for j, v in enumerate(t)]
        return t

    def head(t, w, e):
        return t[:, w * PW + e * Dh:w * PW + (e + 1) * Dh]

    def scores(ts):
        return [_dot_nt(head(t, 0, e), head(t, 1, e)) for e in range(2) for t in ts]

    def softmax(s, which):
        n = s.shape[0]
        f = fill[which, 0:n, 0:n]
        s = jnp.where(f == 0.0, s * scale, f)
        e = jnp.exp(s - jnp.max(s, axis=-1, keepdims=True))
        l = jnp.sum(e, axis=-1, keepdims=True)
        r = pl.reciprocal(l, approx=True)
        r = r * (2.0 - l * r)
        return (e * r).astype(BF16)

    def pv(g, ts, ps, paired):
        for e in range(2):
            o1, o2 = (_dot(ps[2 * e + j], head(t, 2, e)) for j, t in enumerate(ts))
            at = slice(g * PW + e * Dh, g * PW + (e + 1) * Dh)
            set_mem(obuf, at, o1[:2 * M], o2[:2 * M])
            if paired:
                set_pair(obuf, at, o1[2 * M:RH], o2[2 * M:RH], o1[RH:], o2[RH:])
            else:
                set_single(obuf, at, o1[2 * M:], o2[2 * M:])

    def weight_sums(raw, extra, idx, rows):
        for c in range(0, raw.shape[-1], 128):
            cols = slice(c, c + 128)
            parts = _strassen_rhs(*(_unpack(raw[idx + (k, rows, cols)]) for k in range(4)))
            for ref, k, j in ((extra, 0, 0), (extra, 1, 5), (extra, 2, 6), (raw, 1, 2), (raw, 2, 3)):
                ref[idx + (k, rows, cols)] = _pack(parts[j])

    def operand(raw, extra, idx, k, cols=slice(None)):
        ref, j = ((extra, 0), (raw, 0), (raw, 1), (raw, 2), (raw, 3), (extra, 1), (extra, 2))[k]
        return _halves(ref[idx + (j, slice(None), cols)])

    def prepare_ffn_weights(part):
        for r in range(0, DH // 2, 8):
            weight_sums(wgu, wgu_sum, (part // 2, part % 2), slice(r, r + 8))
        for r in range(0, FQ // 4, 8):
            weight_sums(wd, wd_sum, (part // 2,),
                        pl.ds(pl.multiple_of(part % 2 * (FQ // 4) + r, 8), 8))

    def block_product(lhs, raw, extra, idx, cols):
        return _strassen_out([_dot(_halves(lhs[k]), operand(raw, extra, idx, k, cols))
                              for k in range(7)])

    def ffn_in():
        y = _layernorm(rbuf[...])
        parts = _strassen_lhs(y[:L, :DH], y[:L, DH:], y[L:, :DH], y[L:, DH:])
        for i, part in enumerate(parts):
            fbuf[i] = _words(part)

    def gate_up(chunk):
        p, c = divmod(chunk, NF)
        cols = slice(c * FC, (c + 1) * FC)
        gate = block_product(fbuf, wgu, wgu_sum, (p, 0), cols)
        up = block_product(fbuf, wgu, wgu_sum, (p, 1), cols)
        h = [jax.nn.gelu(a, approximate=True) * u for a, u in zip(gate, up)]
        for i, part in enumerate(_strassen_lhs(*h)):
            gbuf[i, :, p * FQ + c * FC:p * FQ + (c + 1) * FC] = _words(part)

    def down(c0, c1):
        out = _strassen_out([
            _dot(_halves(gbuf[k, :, 0:FQ]), operand(wd, wd_sum, (0,), k, slice(c0, c1)))
            + _dot(_halves(gbuf[k, :, FQ:]), operand(wd, wd_sum, (1,), k, slice(c0, c1)))
            for k in range(7)])
        for k, part in enumerate(out):
            at = (slice(k // 2 * L, (k // 2 + 1) * L), slice(k % 2 * DH + c0, k % 2 * DH + c1))
            facc[at] = rbuf[at] + part

    def attention(paired, pre_slot, which, with_ffn=False):
        cur = qkv(0, paired, pre_slot)
        G0 = cfg.get("G0", 0)
        if with_ffn and G0 == 0:
            ffn_in()
        for g in range(NG):
            ss = scores(cur)
            nxt = None if g + 1 == NG else qkv(g + 1, paired, pre_slot)
            if with_ffn and G0 and g == G0 - 1:
                ffn_in()
            if with_ffn and g + 1 < NG:
                n = NG - 1 - G0
                for chunk in range(max(g - G0, 0) * 2 * NF // n, max(g + 1 - G0, 0) * 2 * NF // n):
                    gate_up(chunk)
            elif with_ffn:
                down(0, DH // 2)
            pv(g, cur, [softmax(s, which) for s in ss], paired)
            cur = nxt
        if with_ffn:
            down(DH // 2, DH)

    def out_proj(paired):
        return jnp.concatenate(
            project(obuf, lambda k: operand(wo, wo_sum, (), k), paired), axis=1)

    every = slice(None)

    def set_tokens(t2, t1=None):
        y2 = _layernorm(t2)
        if t1 is None:
            set_single(hbuf, every, y2[:, :DH], y2[:, DH:])
        else:
            y1 = _layernorm(t1)
            set_pair(hbuf, every, y2[:, :DH], y2[:, DH:], y1[:, :DH], y1[:, DH:])

    def set_memory(m1, m2):
        m = jnp.concatenate([m1, m2], axis=0)
        set_mem(hbuf, every, m[:, :DH], m[:, DH:])

    def single_layer_step(which):
        attention(False, None, which)
        a = out_proj(False)
        return a[2 * M:RH], a[0:M], a[M:2 * M]

    def ffn_step():
        ffn_in()
        for chunk in range(2 * NF):
            gate_up(chunk)
        down(0, DH)

    def full_step(t, pre_slot, with_ffn, next_from_pre):
        attention(True, pre_slot, 0, with_ffn)
        if with_ffn:
            x2buf[(t + 1) % 2] = facc[:L, :]
            ov[(t - 3) % 2] = facc[L:, :].astype(BF16)
        if cfg.get("TL"):
            a = out_proj(True)
        set_tokens(x2buf[(t + 1) % 2],
                   None if next_from_pre else x_rows(jnp.minimum(t + 1, n_seg - 1)))
        if not cfg.get("TL"):
            a = out_proj(True)
        set_memory(a[0:M], a[M:2 * M])
        rbuf[0:L, :] = x_rows(t) + a[RH:R]
        rbuf[L:, :] = x2buf[t % 2] + a[2 * M:RH]

    def out_copy(s):
        return pltpu.make_async_copy(ov.at[s % 2], out_hbm.at[seg(s)], sem_o)

    if cfg.get("ONLY"):
        for _, cp in late_cps:
            cp.wait()
        lax.fori_loop(LAG + NP, n_seg, lambda t, c: full_step(t, None, True, False), None)
        return
    mem0 = mem0_ref[...].astype(F32)
    zero_mem = jnp.zeros_like(mem0)
    set_memory(mem0, zero_mem)
    for (cp,) in wo_cps:
        cp.wait()

    def prepare_wo(i, c):
        for r in range(0, KO // 8, 8):
            weight_sums(wo, wo_sum, (), pl.ds(pl.multiple_of(i * (KO // 8) + r, 8), 8))
        return c
    lax.fori_loop(0, 4, prepare_wo, 0)

    def fill_step(s, c):
        set_tokens(x_rows(s))
        a, m1, _ = single_layer_step(1)
        rbuf[seg(s), :] = x_rows(s) + a
        set_memory(m1, jnp.where(s == LAG - 1, mem0_ref[...].astype(F32), 0.0))
        return c
    lax.fori_loop(0, LAG, fill_step, 0)

    for cps in ffn_cps:
        for cp in cps:
            cp.wait()
    x_cp1.wait()
    lax.fori_loop(0, 4, lambda i, c: prepare_ffn_weights(i), None)
    ffn_step()
    x2buf[0] = facc[:L, :]
    x2buf[1] = facc[L:, :]
    set_tokens(facc[:L, :])
    full_step(LAG, 0, False, True)

    def steady(from_pre):
        def step(t, c):
            if cfg.get("DT"):
                pl.when(t > LAG + 2)(lambda: out_copy(t - 5).wait())
                pl.when(t > LAG + 1)(lambda: out_copy(t - 4).start())
            full_step(t, t - LAG if from_pre else None, True, from_pre)
            if not cfg.get("DT"):
                pl.when(t > LAG + 1)(lambda: out_copy(t - 4).wait())
                out_copy(t - 3).start()
            return c
        return step
    lax.fori_loop(LAG + 1, LAG + NP, steady(True), 0)
    set_tokens(x2buf[NP % 2], x_rows(LAG + NP))
    lax.fori_loop(LAG + NP, n_seg, steady(False), 0)

    ffn_step()
    x2buf[(n_seg - 1) % 2] = facc[:L, :]
    ov[(n_seg - 3) % 2] = facc[L:, :].astype(BF16)
    out_copy(n_seg - 4).wait()
    out_copy(n_seg - 3).start()
    for k in range(1, 5):
        hbuf[k, 0:M // 2, :] = jnp.zeros((M // 2, DH), U32)

    def drain_step(i, c):
        s = n_seg - LAG + i
        set_tokens(x2buf[s % 2])
        a, _, m2 = single_layer_step(0)
        rbuf[seg(i), :] = x2buf[s % 2] + a
        set_memory(zero_mem, m2)
        return c
    lax.fori_loop(0, LAG, drain_step, 0)

    ffn_step()
    out_copy(n_seg - 3).wait()
    ov[0] = facc[:L, :].astype(BF16)
    ov[1] = facc[L:, :].astype(BF16)
    out_copy(n_seg - 2).start()
    out_copy(n_seg - 1).start()
    out_copy(n_seg - 2).wait()
    out_copy(n_seg - 1).wait()


def build(x, mem0, Wq, Wk, Wv, Wo, L, wg, wu, wd, cfg=None):
    cfg = {"NP": 14, "PF": 4, "when": (0, 1, 2, 3, 4, 5, 6, 6, 7, 7, 8), **(cfg or {})}
    B, S, D = x.shape
    H, Dh = Wq.shape[1], Wq.shape[2]
    M = mem0.shape[1]
    Df = wg.shape[1]
    assert B == 1 and S % (2 * L) == 0
    R = 2 * M + 2 * L
    NG = H // HG
    NP = cfg["NP"]
    FQ = Df // 4
    any_spec = pl.BlockSpec(memory_space=pl.ANY)
    out = pl.pallas_call(
        functools.partial(_body, S=S, D=D, H=H, Dh=Dh, M=M, L=L, Df=Df, cfg=cfg),
        out_shape=jax.ShapeDtypeStruct((S, D), x.dtype),
        in_specs=[any_spec, pl.BlockSpec(memory_space=pltpu.VMEM)] + [any_spec] * 7,
        out_specs=any_spec,
        scratch_shapes=[
            pltpu.VMEM((S, D), BF16),
            pltpu.VMEM((2, L, D), BF16),
            pltpu.VMEM((2, 6, D, Dh), U32),
            pltpu.VMEM((NG // 2, 7, D // 4, 6 * Dh), U32),
            pltpu.VMEM((NG // 2, 7, D // 4, 6 * Dh), U32),
            pltpu.VMEM((4, H * Dh // 4, D // 2), U32),
            pltpu.VMEM((3, H * Dh // 4, D // 2), U32),
            pltpu.VMEM((2, 2, 4, D // 4, FQ), U32),
            pltpu.VMEM((2, 2, 3, D // 4, FQ), U32),
            pltpu.VMEM((2, 4, FQ // 2, D // 2), U32),
            pltpu.VMEM((2, 3, FQ // 2, D // 2), U32),
            pltpu.VMEM((NP // 2, 7, L // 2, D // 2), U32),
            pltpu.VMEM((NP, NG, 2, L // 2, 6 * Dh), U32),
            pltpu.VMEM((7, M + L // 2, D // 2), U32),
            pltpu.VMEM((7, M + L // 2, H * Dh // 2), U32),
            pltpu.VMEM((7, L // 2, D // 2), U32),
            pltpu.VMEM((7, L // 2, Df // 2), U32),
            pltpu.VMEM((2 * L, D), F32),
            pltpu.VMEM((2 * L, D), F32),
            pltpu.VMEM((2, L, D), F32),
            pltpu.VMEM((2, R, R), F32),
            pltpu.SemaphoreType.DMA((2,)),
            pltpu.SemaphoreType.DMA((2,)),
            pltpu.SemaphoreType.DMA((10,)),
            pltpu.SemaphoreType.DMA,
        ],
        compiler_params=pltpu.CompilerParams(vmem_limit_bytes=127 * 2**20),
        name="rmt_geglu",
    )(x.reshape(S, D), mem0.reshape(M, D), Wq, Wk, Wv, Wo.reshape(H * Dh, D), wg, wu, wd)
    return out.reshape(B, S, D)


@functools.partial(jax.jit, static_argnames=("A_seg_len",))
def pallas_interleave_layers__memory_aug_recurrent_mem_tr__glu_gated_geglu__prompt_kernel(
    A_x: jax.Array,
    A_mem0: jax.Array,
    A_Wq: jax.Array,
    A_Wk: jax.Array,
    A_Wv: jax.Array,
    A_Wo: jax.Array,
    A_seg_len: int,
    B_x: jax.Array,
    B_w_gate: jax.Array,
    B_w_up: jax.Array,
    B_w_down: jax.Array,
):
    del B_x
    return build(A_x, A_mem0, A_Wq, A_Wk, A_Wv, A_Wo, int(A_seg_len),
                 B_w_gate, B_w_up, B_w_down, {"PF": 3})
```

```python
import functools

import jax
import jax.numpy as jnp
from jax import lax
import jax.experimental.pallas as pl
import jax.experimental.pallas.tpu as pltpu

F32 = jnp.float32
BF16 = jnp.bfloat16
U32 = jnp.uint32
HG = 4
EPS = 1e-5
NEG = -1000000000.0


def _layernorm(x):
    m = jnp.mean(x, axis=-1, keepdims=True)
    c = x - m
    v = jnp.mean(c * c, axis=-1, keepdims=True)
    return c * lax.rsqrt(v + EPS)


def _dot(a, b):
    return jnp.dot(a, b, preferred_element_type=F32)


def _dot_nt(a, b):
    return lax.dot_general(a, b, (((1,), (1,)), ((), ())), preferred_element_type=F32)


def _words(x):
    return pltpu.bitcast(x.astype(BF16), U32)


def _halves(w):
    return pltpu.bitcast(w, BF16)


def _unpack(w):
    return pltpu.bitcast(w << 16, F32), pltpu.bitcast(w & U32(0xFFFF0000), F32)


def _strassen_lhs(a11, a12, a21, a22):
    return (a11 + a22, a21 + a22, a11, a22, a11 + a12, a21 - a11, a12 - a22)


def _pack(even, odd):
    return pltpu.bitcast(pltpu.pack_elementwise([even, odd], packed_dtype=BF16), U32)


_SCHEME = (
    "+000+000 ++0+0000+000+000 0000+000",
    "+0000000 +0+++0000000+000 +000-000",
    "0+000+00 0000++0+0-000000 0+000000",
    "00000+00 0+000+-000000-00 0-000+00",
    "00+00000 000000-0+0+++000 00+00000",
    "000000+0 00++00000-+000+0 000000+0",
    "000+000+ 00000000000+0+0+ 0000000+",
    "000+0000 0000000-000000++ 000+000-",
    "+-000000 0000-00000000000 +-000000",
    "+0000+00 0-00+00000000000 0-00+000",
    "0000+-00 0-00000000000000 0000+-00",
    "+0-0+0-0 00000000-000-000 +0-00000",
    "+000+0-0 00--0000+000+000 +0-0-000",
    "0000+0-0 00++000000000000 +0-0-0+0",
    "0++00++0 000000000+000000 00000++0",
    "0++00+00 000000-00+000000 0+000--0",
    "0++00000 000000+000000000 0++00--0",
    "0+0+0000 0000000-00000000 0+0-0000",
    "000-0+00 0000000-00000-00 0+00000-",
    "00000+0+ 0000000000000+00 00000+0-",
    "00+-00+- 00000000000-+000 00+-0000",
    "000-00+- 00000000000+00-0 00+-000+",
    "000000+- 000-0000000000+0 00+-00-+",
    "+0+-0000 000000000000-000 +0+-0000",
    "+00000-+ 000-00000000+000 00+-+000",
    "0000+0+- 000-000000000000 0000+0+-",
)
_U, _V, _W = zip(*(
    [[{"+": 1, "-": -1, "0": 0}[c] for c in part] for part in line.split()] for line in _SCHEME))
NPROD = len(_SCHEME)
_FIRST = tuple(r for r in range(NPROD) if any(_U[r][:4]) and any(_W[r][:4]))


def _signed_sum(signs, values):
    terms = sorted(((s, v) for s, v in zip(signs, values) if s), key=lambda t: -t[0])
    total = terms[0][1] if terms[0][0] > 0 else -terms[0][1]
    for s, v in terms[1:]:
        total = total + v if s > 0 else total - v
    return total


def _quarters(x):
    n = x.shape[1] // 4
    return [x[:, i * n:(i + 1) * n] for i in range(4)]


def _body(x_hbm, mem0_ref, wq_hbm, wk_hbm, wv_hbm, wo_hbm, wg_hbm, wu_hbm, wd_hbm, out_hbm,
          xv, ov, stage, wqkv_even, wqkv_odd, wo, wgu, wd, pre_in, pre, hbuf, obuf,
          fbuf, gbuf, facc, rbuf, x2buf, fill, sem_x, sem_qkv, sem_w, sem_o,
          *, S, D, H, Dh, M, L, Df, cfg):
    n_seg = S // L
    NG = H // HG
    R = 2 * M + 2 * L
    RH = 2 * M + L
    FQ = Df // 4
    FC = 128
    NF = FQ // FC
    DQ = D // 4
    LAG = 2
    NP = cfg["NP"]
    scale = Dh ** -0.5

    def seg(s, rows=L):
        return pl.ds(pl.multiple_of(s * rows, rows), rows)

    XA = (LAG + NP) * L
    x_cp0 = pltpu.make_async_copy(x_hbm.at[0:XA], xv.at[0:XA], sem_x.at[0])
    x_cp1 = pltpu.make_async_copy(x_hbm.at[XA:S], xv.at[XA:S], sem_x.at[1])

    def qkv_copies(g, par):
        return [pltpu.make_async_copy(src.bitcast(U32).at[:, g + side * NG, :],
                                      stage.at[par, 2 * w + side], sem_qkv.at[par])
                for w, src in enumerate((wq_hbm, wk_hbm, wv_hbm)) for side in range(2)]

    def quarter_copies(src, dst, i, sem):
        nr, nc = dst.shape[1:]
        return [pltpu.make_async_copy(src.bitcast(U32).at[i * nr:(i + 1) * nr, j * nc:(j + 1) * nc],
                                      dst.at[4 * i + j], sem_w.at[sem]) for j in range(4)]

    def wo_copies(i):
        side, e = divmod(i, 2)
        return [pltpu.make_async_copy(
            wo_hbm.bitcast(U32).at[pl.ds((2 * (g + side * NG) + e) * (Dh // 2), Dh // 2),
                                   j * DQ:(j + 1) * DQ],
            wo.at[4 * i + j, pl.ds(g * (Dh // 2), Dh // 2)], sem_w.at[i])
            for g in range(NG) for j in range(4)]

    wo_cps = [wo_copies(i) for i in range(4)]
    ffn_cps = [quarter_copies(src, dst, 2 * h, 4 + 2 * w + h)
               + quarter_copies(src, dst, 2 * h + 1, 4 + 2 * w + h)
               for w, (src, dst) in enumerate(((wg_hbm, wgu.at[0]), (wu_hbm, wgu.at[1]), (wd_hbm, wd)))
               for h in range(2)]
    late_cps = [(when, cp) for when, cps in zip(cfg["when"], wo_cps + ffn_cps + [[x_cp1]]) for cp in cps]
    x_cp0.start()
    for cp in qkv_copies(0, 0):
        cp.start()

    row = lax.broadcasted_iota(jnp.int32, (R, R), 0)
    col = lax.broadcasted_iota(jnp.int32, (R, R), 1)
    allowed = jnp.where((row < 2 * M) | (row >= col), 0.0, NEG)
    fill[0] = jnp.where(((row >= M) & (row < RH)) == ((col >= M) & (col < RH)), allowed, -jnp.inf)
    fill[1] = jnp.where(((row >= M) & (row < 2 * M)) == ((col >= M) & (col < 2 * M)), allowed, -jnp.inf)

    def set_mem(dst, at, m):
        for r in _FIRST:
            dst[r, 0:M, at] = _words(_signed_sum(_U[r][:4], m))

    def set_pair(dst, row0, at, a, b):
        for r in range(NPROD):
            dst[r, row0:row0 + L // 2, at] = _words(_signed_sum(_U[r], list(a) + list(b)))

    def set_single(dst, at, a):
        for r in _FIRST:
            dst[r, M:RH // 2, at] = _words(_signed_sum(_U[r][:4], a))

    def block_product(lhs, rhs, row0=0):
        m = [_dot(lhs(r, row0), rhs(r)) for r in range(NPROD)]
        return [_signed_sum([w[k] for w in _W], m) for k in range(8)]

    def project(lhs, rhs, paired):
        if not paired:
            m = [_dot(_halves(lhs[r]), rhs(r)) for r in _FIRST]
            return [_signed_sum([_W[r][k] for r in _FIRST], m) for k in range(4)]
        m = [_dot(_halves(lhs[r] if r in _FIRST else lhs[r, M:, :]), rhs(r)) for r in range(NPROD)]
        tok = [v[2 * M:] if r in _FIRST else v for r, v in enumerate(m)]
        out = [_signed_sum([w[k] for w in _W], tok) for k in range(8)]
        return [jnp.concatenate(
            [_signed_sum([_W[r][k] for r in _FIRST], [m[r][:2 * M] for r in _FIRST]),
             out[k], out[4 + k]], axis=0) for k in range(4)]

    def x_rows(s):
        return xv[seg(s), :].astype(F32)

    x_cp0.wait()
    for k in range(NP // 2):
        y = _layernorm(xv[(LAG + 2 * k) * L:(LAG + 2 * k + 2) * L, :].astype(F32))
        set_pair(pre_in.at[k], 0, slice(None), _quarters(y[:L]), _quarters(y[L:]))

    wqkv = (wqkv_even, wqkv_odd)
    RC = 8

    def regroup(i, par, which=range(3)):
        for w in which:
            for r0 in range(0, DQ // 2, RC):
                even, odd = (
                    [half for k in range(4) for side in range(2) for half in _unpack(
                        stage[par, 2 * w + side, pl.ds(k * DQ + 2 * r0 + o, RC, stride=2), :])]
                    for o in range(2))
                for r in range(NPROD):
                    wqkv[par][i, r, r0:r0 + RC, w * Dh:(w + 1) * Dh] = _pack(
                        _signed_sum(_V[r], even), _signed_sum(_V[r], odd))

    def precompute(i, par, k):
        out = block_product(lambda r, _: _halves(pre_in[k, r]), lambda r: _halves(wqkv[par][i, r]))
        for j, part in enumerate(out):
            pre[2 * k + j // 4, 2 * i + par, j % 4] = _words(part)

    def wait_qkv(par):
        pltpu.make_async_copy(stage.at[par], stage.at[par], sem_qkv.at[par]).wait()

    def start_late(g):
        for when, cp in late_cps:
            if isinstance(g, int):
                if when == g:
                    cp.start()
            elif 0 < when < NG - 1:
                pl.when(g == when)(cp.start)

    def load_step(i, par, first=0):
        g = 2 * i + par
        wait_qkv(1 - par)

        @pl.when(g + 2 < NG)
        def _():
            for cp in qkv_copies(g + 2, par):
                cp.start()
        start_late(g)
        for k in range(first, NP // 2):
            precompute(i, par, k)
            if True and (k - first) % 2 == 1 and (k - first) // 2 < 3:
                regroup(i + par, 1 - par, [(k - first) // 2])
        done = (NP // 2 - first) // 2
        regroup(i + par, 1 - par, range(done, 3))

    assert NP % 2 == 0
    wait_qkv(0)
    for cp in qkv_copies(1, 1):
        cp.start()
    regroup(0, 0)
    PF = min(cfg["PF"], NP // 2)
    for k in range(PF):
        precompute(0, 0, k)
    load_step(0, 0, PF)

    def load_pair(i, c):
        load_step(i, 1)
        load_step(i + 1, 0)
        return c
    lax.fori_loop(0, NG // 2 - 1, load_pair, 0)
    start_late(NG - 1)
    for k in range(NP // 2):
        precompute(NG // 2 - 1, 1, k)
    start_late(NG)

    def qkv(g, paired, pre_slot):
        t = project(hbuf, lambda k: _halves(wqkv[g % 2][g // 2, k]), paired and pre_slot is None)
        t = [v.astype(BF16) for v in t]
        if pre_slot is not None:
            t = [jnp.concatenate([v, _halves(pre[pre_slot, g, j])], axis=0) for j, v in enumerate(t)]
        return t

    def scores(ts):
        return [_dot_nt(t[:, 0:Dh], t[:, Dh:2 * Dh]) for t in ts]

    def softmax(s, which):
        n = s.shape[0]
        f = fill[which, 0:n, 0:n]
        s = jnp.where(f == 0.0, s * scale, f)
        e = jnp.exp(s - jnp.max(s, axis=-1, keepdims=True))
        l = jnp.sum(e, axis=-1, keepdims=True)
        r = pl.reciprocal(l, approx=True)
        r = r * (2.0 - l * r)
        return (e * r).astype(BF16)

    def pv(g, ts, ps, paired):
        o = [_dot(p, t[:, 2 * Dh:]) for p, t in zip(ps, ts)]
        at = slice(g * Dh, (g + 1) * Dh)
        set_mem(obuf, at, [v[:2 * M] for v in o])
        if paired:
            set_pair(obuf, M, at, [v[2 * M:RH] for v in o], [v[RH:] for v in o])
        else:
            set_single(obuf, at, [v[2 * M:] for v in o])

    def combine_weights(ref, row0, n_rows):
        for r0 in range(0, n_rows, 8):
            rows = pl.ds(pl.multiple_of(row0 + r0, 8), 8)
            for c in range(0, ref.shape[-1], 128):
                even, odd = zip(*(_unpack(ref[k, rows, c:c + 128]) for k in range(16)))
                for r in range(NPROD):
                    ref[r, rows, c:c + 128] = _pack(_signed_sum(_V[r], even), _signed_sum(_V[r], odd))

    def ffn_in():
        y = _layernorm(rbuf[...])
        set_pair(fbuf, 0, slice(None), _quarters(y[:L]), _quarters(y[L:]))

    def gate_up(c):
        cols = slice(c * FC, (c + 1) * FC)
        gate, up = (block_product(lambda r, _: _halves(fbuf[r]),
                                  lambda r: _halves(wgu[w, r, :, cols])) for w in range(2))
        h = [jax.nn.gelu(a, approximate=True) * u for a, u in zip(gate, up)]
        set_pair(gbuf, 0, cols, h[:4], h[4:])

    def down(c0, c1):
        out = block_product(lambda r, _: _halves(gbuf[r]), lambda r: _halves(wd[r, :, c0:c1]))
        for k, part in enumerate(out):
            at = (slice(k // 4 * L, (k // 4 + 1) * L), slice(k % 4 * DQ + c0, k % 4 * DQ + c1))
            facc[at] = rbuf[at] + part

    def attention(paired, pre_slot, which, with_ffn=False):
        cur = qkv(0, paired, pre_slot)
        if with_ffn:
            ffn_in()
        for g in range(NG):
            ss = scores(cur)
            nxt = None if g + 1 == NG else qkv(g + 1, paired, pre_slot)
            if with_ffn and g + 1 < NG:
                for c in range(g * NF // (NG - 1), (g + 1) * NF // (NG - 1)):
                    gate_up(c)
            elif with_ffn:
                down(0, DQ // 2)
            pv(g, cur, [softmax(s, which) for s in ss], paired)
            cur = nxt
        if with_ffn:
            down(DQ // 2, DQ)

    def out_proj(paired):
        return jnp.concatenate(
            project(obuf, lambda r: _halves(wo[r]), paired), axis=1)

    every = slice(None)

    def set_tokens(t2, t1=None):
        y2 = _layernorm(t2)
        if t1 is None:
            set_single(hbuf, every, _quarters(y2))
        else:
            set_pair(hbuf, M, every, _quarters(y2), _quarters(_layernorm(t1)))

    def set_memory(m1, m2):
        m = jnp.concatenate([m1, m2], axis=0)
        set_mem(hbuf, every, _quarters(m))

    def single_layer_step(which):
        attention(False, None, which)
        a = out_proj(False)
        return a[2 * M:RH], a[0:M], a[M:2 * M]

    def ffn_step():
        ffn_in()
        for c in range(NF):
            gate_up(c)
        down(0, DQ)

    def full_step(t, pre_slot, with_ffn, next_from_pre):
        attention(True, pre_slot, 0, with_ffn)
        if with_ffn:
            x2buf[(t + 1) % 2] = facc[:L, :]
            ov[(t - 3) % 2] = facc[L:, :].astype(BF16)
        if cfg.get("TL"):
            a = out_proj(True)
        set_tokens(x2buf[(t + 1) % 2],
                   None if next_from_pre else x_rows(jnp.minimum(t + 1, n_seg - 1)))
        if not cfg.get("TL"):
            a = out_proj(True)
        set_memory(a[0:M], a[M:2 * M])
        rbuf[0:L, :] = x_rows(t) + a[RH:R]
        rbuf[L:, :] = x2buf[t % 2] + a[2 * M:RH]

    def out_copy(s):
        return pltpu.make_async_copy(ov.at[s % 2], out_hbm.at[seg(s)], sem_o)

    if cfg.get("ONLY"):
        for _, cp in late_cps:
            cp.wait()
        lax.fori_loop(LAG + NP, n_seg, lambda t, c: full_step(t, None, True, False), None)
        return
    mem0 = mem0_ref[...].astype(F32)
    zero_mem = jnp.zeros_like(mem0)
    set_memory(mem0, zero_mem)
    for cps in wo_cps:
        for cp in cps:
            cp.wait()
    lax.fori_loop(0, NG, lambda i, c: combine_weights(wo, i * (Dh // 2), Dh // 2), None)

    def fill_step(s, c):
        set_tokens(x_rows(s))
        a, m1, _ = single_layer_step(1)
        rbuf[seg(s), :] = x_rows(s) + a
        set_memory(m1, jnp.where(s == LAG - 1, mem0_ref[...].astype(F32), 0.0))
        return c
    lax.fori_loop(0, LAG, fill_step, 0)

    for cps in ffn_cps:
        for cp in cps:
            cp.wait()
    x_cp1.wait()
    for w in range(2):
        lax.fori_loop(0, DQ // 32, lambda i, c, w=w: combine_weights(wgu.at[w], i * 16, 16), None)
    lax.fori_loop(0, FQ // 64, lambda i, c: combine_weights(wd, i * 32, 32), None)
    ffn_step()
    x2buf[0] = facc[:L, :]
    x2buf[1] = facc[L:, :]
    set_tokens(facc[:L, :])
    full_step(LAG, 0, False, True)

    def steady(from_pre):
        def step(t, c):
            if cfg.get("DT"):
                pl.when(t > LAG + 2)(lambda: out_copy(t - 5).wait())
                pl.when(t > LAG + 1)(lambda: out_copy(t - 4).start())
            full_step(t, t - LAG if from_pre else None, True, from_pre)
            if not cfg.get("DT"):
                pl.when(t > LAG + 1)(lambda: out_copy(t - 4).wait())
                out_copy(t - 3).start()
            return c
        return step
    lax.fori_loop(LAG + 1, LAG + NP, steady(True), 0)
    set_tokens(x2buf[NP % 2], x_rows(LAG + NP))
    lax.fori_loop(LAG + NP, n_seg, steady(False), 0)

    ffn_step()
    x2buf[(n_seg - 1) % 2] = facc[:L, :]
    ov[(n_seg - 3) % 2] = facc[L:, :].astype(BF16)
    out_copy(n_seg - 4).wait()
    out_copy(n_seg - 3).start()
    for r in _FIRST:
        hbuf[r, 0:M // 2, :] = jnp.zeros((M // 2, DQ), U32)

    def drain_step(i, c):
        s = n_seg - LAG + i
        set_tokens(x2buf[s % 2])
        a, _, m2 = single_layer_step(0)
        rbuf[seg(i), :] = x2buf[s % 2] + a
        set_memory(zero_mem, m2)
        return c
    lax.fori_loop(0, LAG, drain_step, 0)

    ffn_step()
    out_copy(n_seg - 3).wait()
    ov[0] = facc[:L, :].astype(BF16)
    ov[1] = facc[L:, :].astype(BF16)
    out_copy(n_seg - 2).start()
    out_copy(n_seg - 1).start()
    out_copy(n_seg - 2).wait()
    out_copy(n_seg - 1).wait()


def build(x, mem0, Wq, Wk, Wv, Wo, L, wg, wu, wd, cfg=None):
    cfg = {"NP": 14, "PF": 4, "when": (0, 1, 2, 3, 4, 5, 6, 6, 7, 7, 8), **(cfg or {})}
    B, S, D = x.shape
    H, Dh = Wq.shape[1], Wq.shape[2]
    M = mem0.shape[1]
    Df = wg.shape[1]
    assert B == 1 and S % (2 * L) == 0
    R = 2 * M + 2 * L
    NG = H // HG
    NP = cfg["NP"]
    FQ = Df // 4
    any_spec = pl.BlockSpec(memory_space=pl.ANY)
    out = pl.pallas_call(
        functools.partial(_body, S=S, D=D, H=H, Dh=Dh, M=M, L=L, Df=Df, cfg=cfg),
        out_shape=jax.ShapeDtypeStruct((S, D), x.dtype),
        in_specs=[any_spec, pl.BlockSpec(memory_space=pltpu.VMEM)] + [any_spec] * 7,
        out_specs=any_spec,
        scratch_shapes=[
            pltpu.VMEM((S, D), BF16),
            pltpu.VMEM((2, L, D), BF16),
            pltpu.VMEM((2, 6, D, Dh), U32),
            pltpu.VMEM((NG // 2, NPROD, D // 8, 3 * Dh), U32),
            pltpu.VMEM((NG // 2, NPROD, D // 8, 3 * Dh), U32),
            pltpu.VMEM((NPROD, H * Dh // 8, D // 4), U32),
            pltpu.VMEM((2, NPROD, D // 8, FQ), U32),
            pltpu.VMEM((NPROD, FQ // 2, D // 4), U32),
            pltpu.VMEM((NP // 2, NPROD, L // 2, D // 4), U32),
            pltpu.VMEM((NP, NG, HG, L // 2, 3 * Dh), U32),
            pltpu.VMEM((NPROD, M + L // 2, D // 4), U32),
            pltpu.VMEM((NPROD, M + L // 2, H * Dh // 4), U32),
            pltpu.VMEM((NPROD, L // 2, D // 4), U32),
            pltpu.VMEM((NPROD, L // 2, FQ), U32),
            pltpu.VMEM((2 * L, D), F32),
            pltpu.VMEM((2 * L, D), F32),
            pltpu.VMEM((2, L, D), F32),
            pltpu.VMEM((2, R, R), F32),
            pltpu.SemaphoreType.DMA((2,)),
            pltpu.SemaphoreType.DMA((2,)),
            pltpu.SemaphoreType.DMA((10,)),
            pltpu.SemaphoreType.DMA,
        ],
        compiler_params=pltpu.CompilerParams(vmem_limit_bytes=127 * 2**20),
        name="rmt_geglu",
    )(x.reshape(S, D), mem0.reshape(M, D), Wq, Wk, Wv, Wo.reshape(H * Dh, D), wg, wu, wd)
    return out.reshape(B, S, D)


@functools.partial(jax.jit, static_argnames=("A_seg_len",))
def pallas_interleave_layers__memory_aug_recurrent_mem_tr__glu_gated_geglu__prompt_kernel(
    A_x: jax.Array,
    A_mem0: jax.Array,
    A_Wq: jax.Array,
    A_Wk: jax.Array,
    A_Wv: jax.Array,
    A_Wo: jax.Array,
    A_seg_len: int,
    B_x: jax.Array,
    B_w_gate: jax.Array,
    B_w_up: jax.Array,
    B_w_down: jax.Array,
):
    del B_x
    return build(A_x, A_mem0, A_Wq, A_Wk, A_Wv, A_Wo, int(A_seg_len),
                 B_w_gate, B_w_up, B_w_down, {"PF": 3})
```

```python
import functools

import jax
import jax.numpy as jnp
from jax import lax
import jax.experimental.pallas as pl
import jax.experimental.pallas.tpu as pltpu

F32 = jnp.float32
BF16 = jnp.bfloat16
U32 = jnp.uint32
HG = 4
EPS = 1e-5
NEG = -1000000000.0


def _layernorm(x):
    m = jnp.mean(x, axis=-1, keepdims=True)
    c = x - m
    v = jnp.mean(c * c, axis=-1, keepdims=True)
    return c * lax.rsqrt(v + EPS)


def _dot(a, b):
    return jnp.dot(a, b, preferred_element_type=F32)


def _dot_nt(a, b):
    return lax.dot_general(a, b, (((1,), (1,)), ((), ())), preferred_element_type=F32)


def _words(x):
    return pltpu.bitcast(x.astype(BF16), U32)


def _halves(w):
    return pltpu.bitcast(w, BF16)


def _unpack(w):
    return pltpu.bitcast(w << 16, F32), pltpu.bitcast(w & U32(0xFFFF0000), F32)


def _strassen_lhs(a11, a12, a21, a22):
    return (a11 + a22, a21 + a22, a11, a22, a11 + a12, a21 - a11, a12 - a22)


def _pack(even, odd):
    return pltpu.bitcast(pltpu.pack_elementwise([even, odd], packed_dtype=BF16), U32)


_SCHEME = (
    "+000+000 ++0+0000+000+000 0000+000",
    "+0000000 +0+++0000000+000 +000-000",
    "0+000+00 0000++0+0-000000 0+000000",
    "00000+00 0+000+-000000-00 0-000+00",
    "00+00000 000000-0+0+++000 00+00000",
    "000000+0 00++00000-+000+0 000000+0",
    "000+000+ 00000000000+0+0+ 0000000+",
    "000+0000 0000000-000000++ 000+000-",
    "+-000000 0000-00000000000 +-000000",
    "+0000+00 0-00+00000000000 0-00+000",
    "0000+-00 0-00000000000000 0000+-00",
    "+0-0+0-0 00000000-000-000 +0-00000",
    "+000+0-0 00--0000+000+000 +0-0-000",
    "0000+0-0 00++000000000000 +0-0-0+0",
    "0++00++0 000000000+000000 00000++0",
    "0++00+00 000000-00+000000 0+000--0",
    "0++00000 000000+000000000 0++00--0",
    "0+0+0000 0000000-00000000 0+0-0000",
    "000-0+00 0000000-00000-00 0+00000-",
    "00000+0+ 0000000000000+00 00000+0-",
    "00+-00+- 00000000000-+000 00+-0000",
    "000-00+- 00000000000+00-0 00+-000+",
    "000000+- 000-0000000000+0 00+-00-+",
    "+0+-0000 000000000000-000 +0+-0000",
    "+00000-+ 000-00000000+000 00+-+000",
    "0000+0+- 000-000000000000 0000+0+-",
)
_U, _V, _W = zip(*(
    [[{"+": 1, "-": -1, "0": 0}[c] for c in part] for part in line.split()] for line in _SCHEME))
NPROD = len(_SCHEME)
_FIRST = tuple(r for r in range(NPROD) if any(_U[r][:4]) and any(_W[r][:4]))


def _signed_sum(signs, values):
    terms = sorted(((s, v) for s, v in zip(signs, values) if s), key=lambda t: -t[0])
    total = terms[0][1] if terms[0][0] > 0 else -terms[0][1]
    for s, v in terms[1:]:
        total = total + v if s > 0 else total - v
    return total


def _quarters(x):
    n = x.shape[1] // 4
    return [x[:, i * n:(i + 1) * n] for i in range(4)]


def _body(x_hbm, mem0_ref, wq_hbm, wk_hbm, wv_hbm, wo_hbm, wg_hbm, wu_hbm, wd_hbm, out_hbm,
          xv, ov, stage, wqkv_even, wqkv_odd, wo, wgu, wd, pre_in, pre, hbuf, obuf,
          fbuf, gbuf, facc, rbuf, x2buf, fill, sem_x, sem_qkv, sem_w, sem_o,
          *, S, D, H, Dh, M, L, Df, cfg):
    n_seg = S // L
    NG = H // HG
    R = 2 * M + 2 * L
    RH = 2 * M + L
    FQ = Df // 4
    FC = 128
    NF = FQ // FC
    DQ = D // 4
    LAG = 2
    NP = cfg["NP"]
    scale = Dh ** -0.5

    def seg(s, rows=L):
        return pl.ds(pl.multiple_of(s * rows, rows), rows)

    XA = (LAG + NP) * L
    x_cp0 = pltpu.make_async_copy(x_hbm.at[0:XA], xv.at[0:XA], sem_x.at[0])
    x_cp1 = pltpu.make_async_copy(x_hbm.at[XA:S], xv.at[XA:S], sem_x.at[1])

    def qkv_copies(g, par):
        return [pltpu.make_async_copy(src.bitcast(U32).at[:, g + side * NG, :],
                                      stage.at[par, 2 * w + side], sem_qkv.at[par])
                for w, src in enumerate((wq_hbm, wk_hbm, wv_hbm)) for side in range(2)]

    def quarter_copies(src, dst, i, sem):
        nr, nc = dst.shape[1:]
        return [pltpu.make_async_copy(src.bitcast(U32).at[i * nr:(i + 1) * nr, j * nc:(j + 1) * nc],
                                      dst.at[4 * i + j], sem_w.at[sem]) for j in range(4)]

    def wo_copies(i):
        side, e = divmod(i, 2)
        return [pltpu.make_async_copy(
            wo_hbm.bitcast(U32).at[pl.ds((2 * (g + side * NG) + e) * (Dh // 2), Dh // 2),
                                   j * DQ:(j + 1) * DQ],
            wo.at[4 * i + j, pl.ds(g * (Dh // 2), Dh // 2)], sem_w.at[i])
            for g in range(NG) for j in range(4)]

    wo_cps = [wo_copies(i) for i in range(4)]
    ffn_cps = [quarter_copies(src, dst, 2 * h, 4 + 2 * w + h)
               + quarter_copies(src, dst, 2 * h + 1, 4 + 2 * w + h)
               for w, (src, dst) in enumerate(((wg_hbm, wgu.at[0]), (wu_hbm, wgu.at[1]), (wd_hbm, wd)))
               for h in range(2)]
    late_cps = [(when, cp) for when, cps in zip(cfg["when"], wo_cps + ffn_cps + [[x_cp1]]) for cp in cps]
    x_cp0.start()
    for cp in qkv_copies(0, 0):
        cp.start()

    row = lax.broadcasted_iota(jnp.int32, (R, R), 0)
    col = lax.broadcasted_iota(jnp.int32, (R, R), 1)
    allowed = jnp.where((row < 2 * M) | (row >= col), 0.0, NEG)
    fill[0] = jnp.where(((row >= M) & (row < RH)) == ((col >= M) & (col < RH)), allowed, -jnp.inf)
    fill[1] = jnp.where(((row >= M) & (row < 2 * M)) == ((col >= M) & (col < 2 * M)), allowed, -jnp.inf)

    def set_mem(dst, at, m):
        for r in _FIRST:
            dst[r, 0:M, at] = _words(_signed_sum(_U[r][:4], m))

    def set_pair(dst, row0, at, a, b):
        for r in range(NPROD):
            dst[r, row0:row0 + L // 2, at] = _words(_signed_sum(_U[r], list(a) + list(b)))

    def set_single(dst, at, a):
        for r in _FIRST:
            dst[r, M:RH // 2, at] = _words(_signed_sum(_U[r][:4], a))

    def block_product(lhs, rhs):
        m = [_dot(lhs(r), rhs(r)) for r in range(NPROD)]
        return [_signed_sum([w[k] for w in _W], m) for k in range(8)]

    def project(lhs, rhs, paired):
        if not paired:
            m = [_dot(_halves(lhs[r]), rhs(r)) for r in _FIRST]
            return [_signed_sum([_W[r][k] for r in _FIRST], m) for k in range(4)]
        m = [_dot(_halves(lhs[r] if r in _FIRST else lhs[r, M:, :]), rhs(r)) for r in range(NPROD)]
        tok = [v[2 * M:] if r in _FIRST else v for r, v in enumerate(m)]
        out = [_signed_sum([w[k] for w in _W], tok) for k in range(8)]
        return [jnp.concatenate(
            [_signed_sum([_W[r][k] for r in _FIRST], [m[r][:2 * M] for r in _FIRST]),
             out[k], out[4 + k]], axis=0) for k in range(4)]

    def x_rows(s):
        return xv[seg(s), :].astype(F32)

    x_cp0.wait()
    for k in range(NP // 2):
        y = _layernorm(xv[(LAG + 2 * k) * L:(LAG + 2 * k + 2) * L, :].astype(F32))
        set_pair(pre_in.at[k], 0, slice(None), _quarters(y[:L]), _quarters(y[L:]))

    wqkv = (wqkv_even, wqkv_odd)
    RC = 8

    def regroup(i, par, which=range(3)):
        for w in which:
            for r0 in range(0, DQ // 2, RC):
                even, odd = (
                    [half for k in range(4) for side in range(2) for half in _unpack(
                        stage[par, 2 * w + side, pl.ds(k * DQ + 2 * r0 + o, RC, stride=2), :])]
                    for o in range(2))
                for r in range(NPROD):
                    wqkv[par][i, r, r0:r0 + RC, w * Dh:(w + 1) * Dh] = _pack(
                        _signed_sum(_V[r], even), _signed_sum(_V[r], odd))

    def lanes(w):
        return slice(w * Dh, (w + 1) * Dh)

    def precompute(i, par, k):
        for w in range(3):
            out = block_product(lambda r: _halves(pre_in[k, r]),
                                lambda r: _halves(wqkv[par][i, r, :, lanes(w)]))
            for j, part in enumerate(out):
                pre[2 * k + j // 4, 2 * i + par, j % 4, :, lanes(w)] = _words(part)

    def wait_qkv(par):
        pltpu.make_async_copy(stage.at[par], stage.at[par], sem_qkv.at[par]).wait()

    def start_late(g):
        for when, cp in late_cps:
            if isinstance(g, int):
                if when == g:
                    cp.start()
            elif 0 < when < NG - 1:
                pl.when(g == when)(cp.start)

    def load_step(i, par, first=0):
        g = 2 * i + par
        wait_qkv(1 - par)

        @pl.when(g + 2 < NG)
        def _():
            for cp in qkv_copies(g + 2, par):
                cp.start()
        start_late(g)
        for k in range(first, NP // 2):
            precompute(i, par, k)
            if (k - first) % 2 == 1 and (k - first) // 2 < 3:
                regroup(i + par, 1 - par, [(k - first) // 2])
        done = (NP // 2 - first) // 2
        regroup(i + par, 1 - par, range(done, 3))

    assert NP % 2 == 0
    wait_qkv(0)
    for cp in qkv_copies(1, 1):
        cp.start()
    regroup(0, 0)
    PF = min(cfg["PF"], NP // 2)
    for k in range(PF):
        precompute(0, 0, k)
    load_step(0, 0, PF)

    def load_pair(i, c):
        load_step(i, 1)
        load_step(i + 1, 0)
        return c
    lax.fori_loop(0, NG // 2 - 1, load_pair, 0)
    start_late(NG - 1)
    for k in range(NP // 2):
        precompute(NG // 2 - 1, 1, k)
    start_late(NG)

    def qkv(g, paired, pre_slot):
        ts = []
        for w in range(3):
            t = project(hbuf, lambda r: _halves(wqkv[g % 2][g // 2, r, :, lanes(w)]),
                        paired and pre_slot is None)
            t = [v.astype(BF16) for v in t]
            if pre_slot is not None:
                t = [jnp.concatenate([v, _halves(pre[pre_slot, g, j, :, lanes(w)])], axis=0)
                     for j, v in enumerate(t)]
            ts.append(t)
        return ts

    def scores(ts):
        return [_dot_nt(q, k) for q, k in zip(ts[0], ts[1])]

    def softmax(s, which):
        n = s.shape[0]
        f = fill[which, 0:n, 0:n]
        s = jnp.where(f == 0.0, s * scale, f)
        e = jnp.exp(s - jnp.max(s, axis=-1, keepdims=True))
        l = jnp.sum(e, axis=-1, keepdims=True)
        r = pl.reciprocal(l, approx=True)
        r = r * (2.0 - l * r)
        return (e * r).astype(BF16)

    def pv(g, ts, ps, paired):
        o = [_dot(p, v) for p, v in zip(ps, ts[2])]
        at = slice(g * Dh, (g + 1) * Dh)
        set_mem(obuf, at, [v[:2 * M] for v in o])
        if paired:
            set_pair(obuf, M, at, [v[2 * M:RH] for v in o], [v[RH:] for v in o])
        else:
            set_single(obuf, at, [v[2 * M:] for v in o])

    def combine_weights(ref, row0, n_rows):
        for r0 in range(0, n_rows, 8):
            rows = pl.ds(pl.multiple_of(row0 + r0, 8), 8)
            for c in range(0, ref.shape[-1], 128):
                even, odd = zip(*(_unpack(ref[k, rows, c:c + 128]) for k in range(16)))
                for r in range(NPROD):
                    ref[r, rows, c:c + 128] = _pack(_signed_sum(_V[r], even), _signed_sum(_V[r], odd))

    def ffn_in():
        y = _layernorm(rbuf[...])
        set_pair(fbuf, 0, slice(None), _quarters(y[:L]), _quarters(y[L:]))

    def gate_up(c):
        cols = slice(c * FC, (c + 1) * FC)
        gate, up = (block_product(lambda r: _halves(fbuf[r]),
                                  lambda r: _halves(wgu[w, r, :, cols])) for w in range(2))
        h = [jax.nn.gelu(a, approximate=True) * u for a, u in zip(gate, up)]
        set_pair(gbuf, 0, cols, h[:4], h[4:])

    def down(c):
        out = block_product(lambda r: _halves(gbuf[r]),
                            lambda r: _halves(wd[r, :, c * FC:(c + 1) * FC]))
        for k, part in enumerate(out):
            c0 = k % 4 * DQ + c * FC
            at = (slice(k // 4 * L, (k // 4 + 1) * L), slice(c0, c0 + FC))
            facc[at] = rbuf[at] + part

    def attention(paired, pre_slot, which, with_ffn=False):
        cur = qkv(0, paired, pre_slot)
        if with_ffn:
            ffn_in()
        for g in range(NG):
            ss = scores(cur)
            nxt = None if g + 1 == NG else qkv(g + 1, paired, pre_slot)
            if with_ffn and g + 1 < NG:
                for c in range(g * NF // (NG - 1), (g + 1) * NF // (NG - 1)):
                    gate_up(c)
            elif with_ffn:
                down(0)
            pv(g, cur, [softmax(s, which) for s in ss], paired)
            cur = nxt
        if with_ffn:
            for c in range(1, DQ // FC):
                down(c)

    def out_proj(paired):
        cols = [project(obuf, lambda r: _halves(wo[r, :, c:c + FC]), paired) for c in range(0, DQ, FC)]
        return jnp.concatenate([t[j] for j in range(4) for t in cols], axis=1)

    every = slice(None)

    def set_tokens(t2, t1=None):
        y2 = _layernorm(t2)
        if t1 is None:
            set_single(hbuf, every, _quarters(y2))
        else:
            set_pair(hbuf, M, every, _quarters(y2), _quarters(_layernorm(t1)))

    def set_memory(m1, m2):
        m = jnp.concatenate([m1, m2], axis=0)
        set_mem(hbuf, every, _quarters(m))

    def single_layer_step(which):
        attention(False, None, which)
        a = out_proj(False)
        return a[2 * M:RH], a[0:M], a[M:2 * M]

    def ffn_step():
        ffn_in()
        for c in range(NF):
            gate_up(c)
        for c in range(DQ // FC):
            down(c)

    def full_step(t, pre_slot, with_ffn, next_from_pre):
        attention(True, pre_slot, 0, with_ffn)
        if with_ffn:
            x2buf[(t + 1) % 2] = facc[:L, :]
            ov[(t - 3) % 2] = facc[L:, :].astype(BF16)
        set_tokens(x2buf[(t + 1) % 2],
                   None if next_from_pre else x_rows(jnp.minimum(t + 1, n_seg - 1)))
        a = out_proj(True)
        set_memory(a[0:M], a[M:2 * M])
        rbuf[0:L, :] = x_rows(t) + a[RH:R]
        rbuf[L:, :] = x2buf[t % 2] + a[2 * M:RH]

    def out_copy(s):
        return pltpu.make_async_copy(ov.at[s % 2], out_hbm.at[seg(s)], sem_o)

    if cfg.get("ONLY"):
        for _, cp in late_cps:
            cp.wait()
        lax.fori_loop(LAG + NP, n_seg, lambda t, c: full_step(t, None, True, False), None)
        return
    mem0 = mem0_ref[...].astype(F32)
    zero_mem = jnp.zeros_like(mem0)
    set_memory(mem0, zero_mem)
    for cps in wo_cps:
        for cp in cps:
            cp.wait()
    lax.fori_loop(0, NG, lambda i, c: combine_weights(wo, i * (Dh // 2), Dh // 2), None)

    def fill_step(s, c):
        set_tokens(x_rows(s))
        a, m1, _ = single_layer_step(1)
        rbuf[seg(s), :] = x_rows(s) + a
        set_memory(m1, jnp.where(s == LAG - 1, mem0_ref[...].astype(F32), 0.0))
        return c
    lax.fori_loop(0, LAG, fill_step, 0)

    for cps in ffn_cps:
        for cp in cps:
            cp.wait()
    x_cp1.wait()
    for w in range(2):
        lax.fori_loop(0, DQ // 32, lambda i, c, w=w: combine_weights(wgu.at[w], i * 16, 16), None)
    lax.fori_loop(0, FQ // 64, lambda i, c: combine_weights(wd, i * 32, 32), None)
    ffn_step()
    x2buf[0] = facc[:L, :]
    x2buf[1] = facc[L:, :]
    set_tokens(facc[:L, :])
    full_step(LAG, 0, False, True)

    def steady(from_pre):
        def step(t, c):
            full_step(t, t - LAG if from_pre else None, True, from_pre)
            pl.when(t > LAG + 1)(lambda: out_copy(t - 4).wait())
            out_copy(t - 3).start()
            return c
        return step
    lax.fori_loop(LAG + 1, LAG + NP, steady(True), 0)
    set_tokens(x2buf[NP % 2], x_rows(LAG + NP))
    lax.fori_loop(LAG + NP, n_seg, steady(False), 0)

    ffn_step()
    x2buf[(n_seg - 1) % 2] = facc[:L, :]
    ov[(n_seg - 3) % 2] = facc[L:, :].astype(BF16)
    out_copy(n_seg - 4).wait()
    out_copy(n_seg - 3).start()
    for r in _FIRST:
        hbuf[r, 0:M // 2, :] = jnp.zeros((M // 2, DQ), U32)

    def drain_step(i, c):
        s = n_seg - LAG + i
        set_tokens(x2buf[s % 2])
        a, _, m2 = single_layer_step(0)
        rbuf[seg(i), :] = x2buf[s % 2] + a
        set_memory(zero_mem, m2)
        return c
    lax.fori_loop(0, LAG, drain_step, 0)

    ffn_step()
    out_copy(n_seg - 3).wait()
    ov[0] = facc[:L, :].astype(BF16)
    ov[1] = facc[L:, :].astype(BF16)
    out_copy(n_seg - 2).start()
    out_copy(n_seg - 1).start()
    out_copy(n_seg - 2).wait()
    out_copy(n_seg - 1).wait()


def build(x, mem0, Wq, Wk, Wv, Wo, L, wg, wu, wd, cfg=None):
    cfg = {"NP": 14, "PF": 3, "when": (0, 1, 2, 3, 4, 5, 6, 6, 7, 7, 8), **(cfg or {})}
    B, S, D = x.shape
    H, Dh = Wq.shape[1], Wq.shape[2]
    M = mem0.shape[1]
    Df = wg.shape[1]
    assert B == 1 and S % (2 * L) == 0
    R = 2 * M + 2 * L
    NG = H // HG
    NP = cfg["NP"]
    FQ = Df // 4
    any_spec = pl.BlockSpec(memory_space=pl.ANY)
    out = pl.pallas_call(
        functools.partial(_body, S=S, D=D, H=H, Dh=Dh, M=M, L=L, Df=Df, cfg=cfg),
        out_shape=jax.ShapeDtypeStruct((S, D), x.dtype),
        in_specs=[any_spec, pl.BlockSpec(memory_space=pltpu.VMEM)] + [any_spec] * 7,
        out_specs=any_spec,
        scratch_shapes=[
            pltpu.VMEM((S, D), BF16),
            pltpu.VMEM((2, L, D), BF16),
            pltpu.VMEM((2, 6, D, Dh), U32),
            pltpu.VMEM((NG // 2, NPROD, D // 8, 3 * Dh), U32),
            pltpu.VMEM((NG // 2, NPROD, D // 8, 3 * Dh), U32),
            pltpu.VMEM((NPROD, H * Dh // 8, D // 4), U32),
            pltpu.VMEM((2, NPROD, D // 8, FQ), U32),
            pltpu.VMEM((NPROD, FQ // 2, D // 4), U32),
            pltpu.VMEM((NP // 2, NPROD, L // 2, D // 4), U32),
            pltpu.VMEM((NP, NG, HG, L // 2, 3 * Dh), U32),
            pltpu.VMEM((NPROD, M + L // 2, D // 4), U32),
            pltpu.VMEM((NPROD, M + L // 2, H * Dh // 4), U32),
            pltpu.VMEM((NPROD, L // 2, D // 4), U32),
            pltpu.VMEM((NPROD, L // 2, FQ), U32),
            pltpu.VMEM((2 * L, D), F32),
            pltpu.VMEM((2 * L, D), F32),
            pltpu.VMEM((2, L, D), F32),
            pltpu.VMEM((2, R, R), F32),
            pltpu.SemaphoreType.DMA((2,)),
            pltpu.SemaphoreType.DMA((2,)),
            pltpu.SemaphoreType.DMA((10,)),
            pltpu.SemaphoreType.DMA,
        ],
        compiler_params=pltpu.CompilerParams(vmem_limit_bytes=127 * 2**20),
        name="rmt_geglu",
    )(x.reshape(S, D), mem0.reshape(M, D), Wq, Wk, Wv, Wo.reshape(H * Dh, D), wg, wu, wd)
    return out.reshape(B, S, D)


@functools.partial(jax.jit, static_argnames=("A_seg_len",))
def pallas_interleave_layers__memory_aug_recurrent_mem_tr__glu_gated_geglu__prompt_kernel(
    A_x: jax.Array,
    A_mem0: jax.Array,
    A_Wq: jax.Array,
    A_Wk: jax.Array,
    A_Wv: jax.Array,
    A_Wo: jax.Array,
    A_seg_len: int,
    B_x: jax.Array,
    B_w_gate: jax.Array,
    B_w_up: jax.Array,
    B_w_down: jax.Array,
):
    del B_x
    return build(A_x, A_mem0, A_Wq, A_Wk, A_Wv, A_Wo, int(A_seg_len),
                 B_w_gate, B_w_up, B_w_down, {})
```

```python
import functools

import jax
import jax.numpy as jnp
from jax import lax
import jax.experimental.pallas as pl
import jax.experimental.pallas.tpu as pltpu

F32 = jnp.float32
BF16 = jnp.bfloat16
U32 = jnp.uint32
HG = 4
PRE_SEGMENTS = 12
START_AT = (1, 2, 3, 4, 6, 6, 7, 7, 8, 8, 8)
EPS = 1e-5
NEG = -1000000000.0
LOG2E = 1.4426950408889634


def _layernorm(x):
    m = jnp.mean(x, axis=-1, keepdims=True)
    c = x - m
    v = jnp.mean(c * c, axis=-1, keepdims=True)
    return c * lax.rsqrt(v + EPS)


def _dot(a, b):
    return jnp.dot(a, b, preferred_element_type=F32)


def _dot_nt(a, b):
    return lax.dot_general(a, b, (((1,), (1,)), ((), ())), preferred_element_type=F32)


def _words(x):
    return pltpu.bitcast(x.astype(BF16), U32)


def _halves(w):
    return pltpu.bitcast(w, BF16)


def _unpack(w):
    return pltpu.bitcast(w << 16, F32), pltpu.bitcast(w & U32(0xFFFF0000), F32)


def _strassen_lhs(a11, a12, a21, a22):
    return (a11 + a22, a21 + a22, a11, a22, a11 + a12, a21 - a11, a12 - a22)


def _pack(even, odd):
    even, odd = (pltpu.bitcast(v, U32) + U32(0x8000) for v in (even, odd))
    return (even >> 16) | (odd & U32(0xFFFF0000))


_SCHEME = (
    "+000+000 ++0+0000+000+000 0000+000",
    "+0000000 +0+++0000000+000 +000-000",
    "0+000+00 0000++0+0-000000 0+000000",
    "00000+00 0+000+-000000-00 0-000+00",
    "00+00000 000000-0+0+++000 00+00000",
    "000000+0 00++00000-+000+0 000000+0",
    "000+000+ 00000000000+0+0+ 0000000+",
    "000+0000 0000000-000000++ 000+000-",
    "+-000000 0000-00000000000 +-000000",
    "+0000+00 0-00+00000000000 0-00+000",
    "0000+-00 0-00000000000000 0000+-00",
    "+0-0+0-0 00000000-000-000 +0-00000",
    "+000+0-0 00--0000+000+000 +0-0-000",
    "0000+0-0 00++000000000000 +0-0-0+0",
    "0++00++0 000000000+000000 00000++0",
    "0++00+00 000000-00+000000 0+000--0",
    "0++00000 000000+000000000 0++00--0",
    "0+0+0000 0000000-00000000 0+0-0000",
    "000-0+00 0000000-00000-00 0+00000-",
    "00000+0+ 0000000000000+00 00000+0-",
    "00+-00+- 00000000000-+000 00+-0000",
    "000-00+- 00000000000+00-0 00+-000+",
    "000000+- 000-0000000000+0 00+-00-+",
    "+0+-0000 000000000000-000 +0+-0000",
    "+00000-+ 000-00000000+000 00+-+000",
    "0000+0+- 000-000000000000 0000+0+-",
)
_U, _V, _W = zip(*(
    [[{"+": 1, "-": -1, "0": 0}[c] for c in part] for part in line.split()] for line in _SCHEME))
NPROD = len(_SCHEME)
_FIRST = tuple(r for r in range(NPROD) if any(_U[r][:4]) and any(_W[r][:4]))


def _signed_sum(signs, values):
    terms = sorted(((s, v) for s, v in zip(signs, values) if s), key=lambda t: -t[0])
    total = terms[0][1] if terms[0][0] > 0 else -terms[0][1]
    for s, v in terms[1:]:
        total = total + v if s > 0 else total - v
    return total


def _share_pairs(table):
    terms = [{i: s for i, s in enumerate(row) if s} for row in table]
    shared, n = [], len(table[0])
    while True:
        count = {}
        for t in terms:
            for i in t:
                for j in t:
                    if i < j:
                        key = (i, j, t[i] * t[j])
                        count[key] = count.get(key, 0) + 1
        best = max(sorted(count), key=count.get, default=None)
        if best is None or count[best] < 2:
            return shared, terms
        i, j, sign = best
        for t in terms:
            if i in t and j in t and t[i] * t[j] == sign:
                t[n] = t.pop(i)
                del t[j]
        shared.append(best)
        n += 1


_V_SHARED = _share_pairs(_V)


def _right_operands(blocks):
    shared, terms = _V_SHARED
    values = list(blocks)
    for i, j, sign in shared:
        values.append(values[i] + values[j] if sign > 0 else values[i] - values[j])
    return [_signed_sum(list(t.values()), [values[i] for i in t]) for t in terms]


def _packed_operands(even, odd, words=None):
    for r, pair in enumerate(zip(_right_operands(even), _right_operands(odd))):
        used = [k for k, sign in enumerate(_V[r]) if sign]
        if len(used) > 1:
            yield _pack(*pair)
            continue
        k = used[0]
        word = words[k] if words else (
            (pltpu.bitcast(even[k], U32) >> 16) | pltpu.bitcast(odd[k], U32))
        yield word if _V[r][k] > 0 else word ^ U32(0x80008000)


def _quarters(x):
    n = x.shape[1] // 4
    return [x[:, i * n:(i + 1) * n] for i in range(4)]


def _body(x_hbm, mem0_ref, wq_hbm, wk_hbm, wv_hbm, wo_hbm, wg_hbm, wu_hbm, wd_hbm, out_hbm,
          xv, ov, stage, wqkv_even, wqkv_odd, wo, wgu, wd, pre_in, pre, hbuf, obuf,
          fbuf, gbuf, facc, rbuf, x2buf, fill, sem_x, sem_qkv, sem_w, sem_o,
          *, S, D, H, Dh, M, L, Df, NP):
    n_seg = S // L
    NG = H // HG
    R = 2 * M + 2 * L
    RH = 2 * M + L
    FQ = Df // 4
    FC = 128
    NF = FQ // FC
    DQ = D // 4
    LAG = 2
    scale = Dh ** -0.5

    def seg(s, rows=L):
        return pl.ds(pl.multiple_of(s * rows, rows), rows)

    XA = (LAG + NP) * L
    x_cp0 = pltpu.make_async_copy(x_hbm.at[0:XA], xv.at[0:XA], sem_x.at[0])
    x_cp1 = pltpu.make_async_copy(x_hbm.at[XA:S], xv.at[XA:S], sem_x.at[1])

    def qkv_copies(g, par):
        return [pltpu.make_async_copy(src.bitcast(U32).at[:, g + side * NG, :],
                                      stage.at[par, 2 * w + side], sem_qkv.at[par])
                for w, src in enumerate((wq_hbm, wk_hbm, wv_hbm)) for side in range(2)]

    def quarter_copies(src, dst, i, sem):
        nr, nc = dst.shape[1:]
        return [pltpu.make_async_copy(src.bitcast(U32).at[i * nr:(i + 1) * nr, j * nc:(j + 1) * nc],
                                      dst.at[4 * i + j], sem_w.at[sem]) for j in range(4)]

    def wo_copies(i):
        side, e = divmod(i, 2)
        return [pltpu.make_async_copy(
            wo_hbm.bitcast(U32).at[pl.ds((2 * (g + side * NG) + e) * (Dh // 2), Dh // 2),
                                   j * DQ:(j + 1) * DQ],
            wo.at[4 * i + j, pl.ds(g * (Dh // 2), Dh // 2)], sem_w.at[i])
            for g in range(NG) for j in range(4)]

    wo_cps = [wo_copies(i) for i in range(4)]
    ffn_cps = [quarter_copies(src, dst, 2 * h, 4 + 2 * w + h)
               + quarter_copies(src, dst, 2 * h + 1, 4 + 2 * w + h)
               for w, (src, dst) in enumerate(((wg_hbm, wgu.at[0]), (wu_hbm, wgu.at[1]), (wd_hbm, wd)))
               for h in range(2)]
    late_cps = [(when, cp) for when, cps in zip(START_AT, wo_cps + ffn_cps + [[x_cp1]]) for cp in cps]
    x_cp0.start()
    for cp in qkv_copies(0, 0):
        cp.start()

    row = lax.broadcasted_iota(jnp.int32, (R, R), 0)
    col = lax.broadcasted_iota(jnp.int32, (R, R), 1)
    allowed = jnp.where((row < 2 * M) | (row >= col), 0.0, NEG / scale)
    fill[0] = jnp.where(((row >= M) & (row < RH)) == ((col >= M) & (col < RH)), allowed, -jnp.inf)
    fill[1] = jnp.where(((row >= M) & (row < 2 * M)) == ((col >= M) & (col < 2 * M)), allowed, -jnp.inf)

    def set_mem(dst, at, m):
        for r in _FIRST:
            dst[r, 0:M, at] = _words(_signed_sum(_U[r][:4], m))

    def set_pair(dst, row0, at, a, b):
        for r in range(NPROD):
            dst[r, row0:row0 + L // 2, at] = _words(_signed_sum(_U[r], list(a) + list(b)))

    def set_single(dst, at, a):
        for r in _FIRST:
            dst[r, M:RH // 2, at] = _words(_signed_sum(_U[r][:4], a))

    def block_product(lhs, rhs):
        m = [_dot(lhs(r), rhs(r)) for r in range(NPROD)]
        return [_signed_sum([w[k] for w in _W], m) for k in range(8)]

    def project(lhs, rhs, paired):
        if not paired:
            m = [_dot(_halves(lhs[r]), rhs(r)) for r in _FIRST]
            return [_signed_sum([_W[r][k] for r in _FIRST], m) for k in range(4)]
        m = [_dot(_halves(lhs[r] if r in _FIRST else lhs[r, M:, :]), rhs(r)) for r in range(NPROD)]
        tok = [v[2 * M:] if r in _FIRST else v for r, v in enumerate(m)]
        out = [_signed_sum([w[k] for w in _W], tok) for k in range(8)]
        return [jnp.concatenate(
            [_signed_sum([_W[r][k] for r in _FIRST], [m[r][:2 * M] for r in _FIRST]),
             out[k], out[4 + k]], axis=0) for k in range(4)]

    def x_rows(s):
        return xv[seg(s), :].astype(F32)

    x_cp0.wait()
    for k in range(NP // 2):
        y = _layernorm(xv[(LAG + 2 * k) * L:(LAG + 2 * k + 2) * L, :].astype(F32))
        set_pair(pre_in.at[k], 0, slice(None), _quarters(y[:L]), _quarters(y[L:]))

    wqkv = (wqkv_even, wqkv_odd)
    RC = 8

    def regroup(i, par):
        for w in range(3):
            for r0 in range(0, DQ // 2, RC):
                even, odd = (
                    [head for k in range(4) for side in range(2) for head in _unpack(
                        stage[par, 2 * w + side, pl.ds(k * DQ + 2 * r0 + o, RC, stride=2), :])]
                    for o in range(2))
                for r, word in enumerate(_packed_operands(even, odd)):
                    wqkv[par][i, r, r0:r0 + RC, w * Dh:(w + 1) * Dh] = word

    def lanes(w):
        return slice(w * Dh, (w + 1) * Dh)

    def precompute(i, par, k):
        for w in range(3):
            out = block_product(lambda r: _halves(pre_in[k, r]),
                                lambda r: _halves(wqkv[par][i, r, :, lanes(w)]))
            for j, part in enumerate(out):
                pre[2 * k + j // 4, 2 * i + par, j % 4, :, lanes(w)] = _words(part)

    def wait_qkv(par):
        pltpu.make_async_copy(stage.at[par], stage.at[par], sem_qkv.at[par]).wait()

    def start_late(g):
        for when, cp in late_cps:
            if isinstance(g, int):
                if when == g:
                    cp.start()
            elif 0 < when < NG - 1:
                pl.when(g == when)(cp.start)

    def load_step(i, par, first=0):
        g = 2 * i + par
        wait_qkv(1 - par)

        @pl.when(g + 2 < NG)
        def _():
            for cp in qkv_copies(g + 2, par):
                cp.start()
        start_late(g)
        for k in range(first, NP // 2):
            precompute(i, par, k)
        regroup(i + par, 1 - par)

    assert NP % 2 == 0
    wait_qkv(0)
    for cp in qkv_copies(1, 1):
        cp.start()
    regroup(0, 0)
    PF = min(3, NP // 2)
    for k in range(PF):
        precompute(0, 0, k)
    load_step(0, 0, PF)

    def load_pair(i, c):
        load_step(i, 1)
        load_step(i + 1, 0)
        return c
    lax.fori_loop(0, NG // 2 - 1, load_pair, 0)
    start_late(NG - 1)
    for k in range(NP // 2):
        precompute(NG // 2 - 1, 1, k)
    start_late(NG)

    def qkv(g, paired, pre_slot):
        ts = []
        for w in range(3):
            t = project(hbuf, lambda r: _halves(wqkv[g % 2][g // 2, r, :, lanes(w)]),
                        paired and pre_slot is None)
            t = [v.astype(BF16) for v in t]
            if pre_slot is not None:
                t = [jnp.concatenate([v, _halves(pre[pre_slot, g, j, :, lanes(w)])], axis=0)
                     for j, v in enumerate(t)]
            ts.append(t)
        return ts

    def scores(ts):
        return [_dot_nt(q, k) for q, k in zip(ts[0], ts[1])]

    def softmax(s, which):
        n = s.shape[0]
        f = fill[which, 0:n, 0:n]
        s = jnp.where(f == 0.0, s, f)
        e = jnp.exp2((s - jnp.max(s, axis=-1, keepdims=True)) * (scale * LOG2E))
        l = jnp.sum(e, axis=-1, keepdims=True)
        r = pl.reciprocal(l, approx=True)
        r = r * (2.0 - l * r)
        return (e * r).astype(BF16)

    def pv(g, ts, ps, paired):
        o = [_dot(p, v) for p, v in zip(ps, ts[2])]
        at = slice(g * Dh, (g + 1) * Dh)
        set_mem(obuf, at, [v[:2 * M] for v in o])
        if paired:
            set_pair(obuf, M, at, [v[2 * M:RH] for v in o], [v[RH:] for v in o])
        else:
            set_single(obuf, at, [v[2 * M:] for v in o])

    def combine_weights(ref, row0, n_rows):
        for r0 in range(0, n_rows, 8):
            rows = pl.ds(pl.multiple_of(row0 + r0, 8), 8)
            for c in range(0, ref.shape[-1], 128):
                words = [ref[k, rows, c:c + 128] for k in range(16)]
                even, odd = zip(*(_unpack(word) for word in words))
                for r, word in enumerate(_packed_operands(even, odd, words)):
                    ref[r, rows, c:c + 128] = word

    def ffn_in():
        y = _layernorm(rbuf[...])
        set_pair(fbuf, 0, slice(None), _quarters(y[:L]), _quarters(y[L:]))

    def gate_up(c):
        cols = slice(c * FC, (c + 1) * FC)
        gate, up = (block_product(lambda r: _halves(fbuf[r]),
                                  lambda r: _halves(wgu[w, r, :, cols])) for w in range(2))
        h = [jax.nn.gelu(a, approximate=True) * u for a, u in zip(gate, up)]
        set_pair(gbuf, 0, cols, h[:4], h[4:])

    def down(c):
        out = block_product(lambda r: _halves(gbuf[r]),
                            lambda r: _halves(wd[r, :, c * FC:(c + 1) * FC]))
        for k, part in enumerate(out):
            c0 = k % 4 * DQ + c * FC
            at = (slice(k // 4 * L, (k // 4 + 1) * L), slice(c0, c0 + FC))
            facc[at] = rbuf[at] + part

    def attention(paired, pre_slot, which, with_ffn=False):
        cur = qkv(0, paired, pre_slot)
        if with_ffn:
            ffn_in()
        for g in range(NG):
            ss = scores(cur)
            nxt = None if g + 1 == NG else qkv(g + 1, paired, pre_slot)
            if with_ffn and g + 1 < NG:
                for c in range(g * NF // (NG - 1), (g + 1) * NF // (NG - 1)):
                    gate_up(c)
            elif with_ffn:
                down(0)
            pv(g, cur, [softmax(s, which) for s in ss], paired)
            cur = nxt
        if with_ffn:
            for c in range(1, DQ // FC):
                down(c)

    def out_proj(paired):
        cols = [project(obuf, lambda r: _halves(wo[r, :, c:c + FC]), paired) for c in range(0, DQ, FC)]
        return jnp.concatenate([t[j] for j in range(4) for t in cols], axis=1)

    every = slice(None)

    def set_tokens(t2, t1=None):
        y2 = _layernorm(t2)
        if t1 is None:
            set_single(hbuf, every, _quarters(y2))
        else:
            set_pair(hbuf, M, every, _quarters(y2), _quarters(_layernorm(t1)))

    def set_memory(m1, m2):
        m = jnp.concatenate([m1, m2], axis=0)
        set_mem(hbuf, every, _quarters(m))

    def single_layer_step(which):
        attention(False, None, which)
        a = out_proj(False)
        return a[2 * M:RH], a[0:M], a[M:2 * M]

    def ffn_step():
        ffn_in()
        for c in range(NF):
            gate_up(c)
        for c in range(DQ // FC):
            down(c)

    def full_step(t, pre_slot, with_ffn, next_from_pre):
        attention(True, pre_slot, 0, with_ffn)
        if with_ffn:
            x2buf[(t + 1) % 2] = facc[:L, :]
            ov[(t - 3) % 2] = facc[L:, :].astype(BF16)
        set_tokens(x2buf[(t + 1) % 2],
                   None if next_from_pre else x_rows(jnp.minimum(t + 1, n_seg - 1)))
        a = out_proj(True)
        set_memory(a[0:M], a[M:2 * M])
        rbuf[0:L, :] = x_rows(t) + a[RH:R]
        rbuf[L:, :] = x2buf[t % 2] + a[2 * M:RH]

    def out_copy(s):
        return pltpu.make_async_copy(ov.at[s % 2], out_hbm.at[seg(s)], sem_o)

    mem0 = mem0_ref[...].astype(F32)
    zero_mem = jnp.zeros_like(mem0)
    set_memory(mem0, zero_mem)
    for cps in wo_cps:
        for cp in cps:
            cp.wait()
    lax.fori_loop(0, NG, lambda i, c: combine_weights(wo, i * (Dh // 2), Dh // 2), None)

    def fill_step(s, c):
        set_tokens(x_rows(s))
        a, m1, _ = single_layer_step(1)
        rbuf[seg(s), :] = x_rows(s) + a
        set_memory(m1, jnp.where(s == LAG - 1, mem0_ref[...].astype(F32), 0.0))
        return c
    lax.fori_loop(0, LAG, fill_step, 0)

    for w in range(3):
        for cp in ffn_cps[2 * w] + ffn_cps[2 * w + 1]:
            cp.wait()
        if w < 2:
            lax.fori_loop(0, DQ // 32, lambda i, c, w=w: combine_weights(wgu.at[w], i * 16, 16), None)
        else:
            lax.fori_loop(0, FQ // 64, lambda i, c: combine_weights(wd, i * 32, 32), None)
    ffn_step()
    x2buf[0] = facc[:L, :]
    x2buf[1] = facc[L:, :]
    set_tokens(facc[:L, :])
    full_step(LAG, 0, False, True)

    def steady(from_pre):
        def step(t, c):
            full_step(t, t - LAG if from_pre else None, True, from_pre)
            pl.when(t > LAG + 1)(lambda: out_copy(t - 4).wait())
            out_copy(t - 3).start()
            return c
        return step
    lax.fori_loop(LAG + 1, LAG + NP, steady(True), 0)
    x_cp1.wait()
    set_tokens(x2buf[NP % 2], x_rows(LAG + NP))
    lax.fori_loop(LAG + NP, n_seg, steady(False), 0)

    ffn_step()
    x2buf[(n_seg - 1) % 2] = facc[:L, :]
    ov[(n_seg - 3) % 2] = facc[L:, :].astype(BF16)
    out_copy(n_seg - 4).wait()
    out_copy(n_seg - 3).start()
    for r in _FIRST:
        hbuf[r, 0:M // 2, :] = jnp.zeros((M // 2, DQ), U32)

    def drain_step(i, c):
        s = n_seg - LAG + i
        set_tokens(x2buf[s % 2])
        a, _, m2 = single_layer_step(0)
        rbuf[seg(i), :] = x2buf[s % 2] + a
        set_memory(zero_mem, m2)
        return c
    lax.fori_loop(0, LAG, drain_step, 0)

    ffn_step()
    out_copy(n_seg - 3).wait()
    ov[0] = facc[:L, :].astype(BF16)
    ov[1] = facc[L:, :].astype(BF16)
    out_copy(n_seg - 2).start()
    out_copy(n_seg - 1).start()
    out_copy(n_seg - 2).wait()
    out_copy(n_seg - 1).wait()


def build(x, mem0, Wq, Wk, Wv, Wo, L, wg, wu, wd):
    B, S, D = x.shape
    H, Dh = Wq.shape[1], Wq.shape[2]
    M = mem0.shape[1]
    Df = wg.shape[1]
    assert B == 1 and S % (2 * L) == 0
    R = 2 * M + 2 * L
    NG = H // HG
    NP = min(PRE_SEGMENTS, (S // L - 4) // 2 * 2)
    FQ = Df // 4
    any_spec = pl.BlockSpec(memory_space=pl.ANY)
    out = pl.pallas_call(
        functools.partial(_body, S=S, D=D, H=H, Dh=Dh, M=M, L=L, Df=Df, NP=NP),
        out_shape=jax.ShapeDtypeStruct((S, D), x.dtype),
        in_specs=[any_spec, pl.BlockSpec(memory_space=pltpu.VMEM)] + [any_spec] * 7,
        out_specs=any_spec,
        scratch_shapes=[
            pltpu.VMEM((S, D), BF16),
            pltpu.VMEM((2, L, D), BF16),
            pltpu.VMEM((2, 6, D, Dh), U32),
            pltpu.VMEM((NG // 2, NPROD, D // 8, 3 * Dh), U32),
            pltpu.VMEM((NG // 2, NPROD, D // 8, 3 * Dh), U32),
            pltpu.VMEM((NPROD, H * Dh // 8, D // 4), U32),
            pltpu.VMEM((2, NPROD, D // 8, FQ), U32),
            pltpu.VMEM((NPROD, FQ // 2, D // 4), U32),
            pltpu.VMEM((NP // 2, NPROD, L // 2, D // 4), U32),
            pltpu.VMEM((NP, NG, HG, L // 2, 3 * Dh), U32),
            pltpu.VMEM((NPROD, M + L // 2, D // 4), U32),
            pltpu.VMEM((NPROD, M + L // 2, H * Dh // 4), U32),
            pltpu.VMEM((NPROD, L // 2, D // 4), U32),
            pltpu.VMEM((NPROD, L // 2, FQ), U32),
            pltpu.VMEM((2 * L, D), F32),
            pltpu.VMEM((2 * L, D), F32),
            pltpu.VMEM((2, L, D), F32),
            pltpu.VMEM((2, R, R), F32),
            pltpu.SemaphoreType.DMA((2,)),
            pltpu.SemaphoreType.DMA((2,)),
            pltpu.SemaphoreType.DMA((10,)),
            pltpu.SemaphoreType.DMA,
        ],
        compiler_params=pltpu.CompilerParams(vmem_limit_bytes=127 * 2**20),
        name="rmt_geglu",
    )(x.reshape(S, D), mem0.reshape(M, D), Wq, Wk, Wv, Wo.reshape(H * Dh, D), wg, wu, wd)
    return out.reshape(B, S, D)


@functools.partial(jax.jit, static_argnames=("A_seg_len",))
def pallas_interleave_layers__memory_aug_recurrent_mem_tr__glu_gated_geglu__prompt_kernel(
    A_x: jax.Array,
    A_mem0: jax.Array,
    A_Wq: jax.Array,
    A_Wk: jax.Array,
    A_Wv: jax.Array,
    A_Wo: jax.Array,
    A_seg_len: int,
    B_x: jax.Array,
    B_w_gate: jax.Array,
    B_w_up: jax.Array,
    B_w_down: jax.Array,
):
    del B_x
    return build(A_x, A_mem0, A_Wq, A_Wk, A_Wv, A_Wo, int(A_seg_len),
                 B_w_gate, B_w_up, B_w_down)
```
